```python
import jax
import jax.numpy as jnp

def _softmax(x, axis=-1):
    return jax.nn.softmax(x, axis=axis)
def _gelu(x):
    return jax.nn.gelu(x, approximate=True)
def _silu(x):
    return jax.nn.silu(x)
def _sigmoid(x):
    return jax.nn.sigmoid(x)
def _layernorm(x, axis=-1, eps=1e-5):
    m = jnp.mean(x, axis=axis, keepdims=True)
    v = jnp.var(x, axis=axis, keepdims=True)
    return (x - m) / jnp.sqrt(v + eps)
def _scatter_add(tgt, idx, src, axis=0):
    return tgt.at[idx].add(src)
def _segment_sum(src, seg, n):
    return jax.ops.segment_sum(src, seg, n)
class _Rng:
    def __init__(self, key):
        self._k = key
    def _next(self):
        self._k, sub = jax.random.split(self._k)
        return sub
    def normal(self, shape):
        return jax.random.normal(self._next(), shape, dtype=jnp.bfloat16)
    def randint(self, lo, hi, shape):
        return jax.random.randint(self._next(), shape, lo, hi, dtype=jnp.int32)
    def uniform(self, shape, lo=0.0, hi=1.0):
        return jax.random.uniform(self._next(), shape, jnp.bfloat16, lo, hi)
    def permutation(self, n):
        return jax.random.permutation(self._next(), n)


kernel_name = 'sequential_preLN__mha_block_cached__moe_arch_mod__decode'

def setup_inputs():
    _rng = _Rng(jax.random.key(int.from_bytes(__import__("os").urandom(4), "little")))
    _w = (lambda a: (lambda t: t.astype(jnp.bfloat16) if jnp.issubdtype(t.dtype, jnp.floating) else t)(jnp.asarray(a)))
    def _A_setup():
        B, Sq, D = 4, 1, 640
        H, Sk, Dh = 32, 8192, 192
        return {
            "x": _w((lambda *s: _rng.normal(s) * 0.05)(B, Sq, D)),
            "k_cache": _w((lambda *s: _rng.normal(s) * 0.05)(B, H, Sk, Dh)),
            "v_cache": _w((lambda *s: _rng.normal(s) * 0.05)(B, H, Sk, Dh)),
            "wq": _w((lambda *s: _rng.normal(s) * 0.05)(D, H * Dh) * (D ** -0.5)),
            "wo": _w((lambda *s: _rng.normal(s) * 0.05)(H * Dh, D) * ((H * Dh) ** -0.5)),
        }
    _A_in = _A_setup()

    def _B_setup():
        B, S, D, F, C = 4, 1, 640, 1536, 1
        return {
            "x": _w((lambda *s: _rng.normal(s) * 0.05)(B, S, D)),
            "w_r": _w((lambda *s: _rng.normal(s) * 0.05)(D)),
            "w_gate": _w((lambda *s: _rng.normal(s) * 0.05)(D, F)),
            "w_up": _w((lambda *s: _rng.normal(s) * 0.05)(D, F)),
            "w_down": _w((lambda *s: _rng.normal(s) * 0.05)(F, D)),
        }
    _B_in = _B_setup()

    return {
        "A_x": _A_in["x"],
        "A_k_cache": _A_in["k_cache"],
        "A_v_cache": _A_in["v_cache"],
        "A_wq": _A_in["wq"],
        "A_wo": _A_in["wo"],
        "B_x": _B_in["x"],
        "B_w_r": _B_in["w_r"],
        "B_w_gate": _B_in["w_gate"],
        "B_w_up": _B_in["w_up"],
        "B_w_down": _B_in["w_down"],
    }

def reference(A_x, A_k_cache, A_v_cache, A_wq, A_wo, B_x, B_w_r, B_w_gate, B_w_up, B_w_down):
    def _A_ref(x, k_cache, v_cache, wq, wo):
        B, Sq, D = x.shape
        H, Dh = 32, 192
        q = (lambda x, *d: x.transpose(*d))((x @ wq).reshape(B, Sq, H, Dh), 0, 2, 1, 3)
        scores = jnp.einsum("bhqd,bhkd->bhqk", q, k_cache) * (Dh ** -0.5)
        p = _softmax(scores, axis=-1)
        o = jnp.einsum("bhqk,bhkd->bhqd", p, v_cache)
        return (lambda x, *d: x.transpose(*d))(o, 0, 2, 1, 3).reshape(B, Sq, H * Dh) @ wo

    def _B_ref(x, w_r, w_gate, w_up, w_down):
        B, S, D = x.shape
        C = 1
        r = x @ w_r
        idx = jnp.argsort(-r, axis=-1)[:, :C]
        idx_e = jnp.repeat(idx.reshape(B, C, 1), D, axis=2)
        x_sel = jnp.take_along_axis(x, idx_e, axis=1)
        g = _silu(x_sel @ w_gate)
        u = x_sel @ w_up
        y = (g * u) @ w_down
        r_sel = _sigmoid(jnp.take_along_axis(r, idx, axis=1))
        y = y * r_sel.reshape(B, C, 1)
        b_off = (jnp.arange(B) * S).reshape(B, 1)
        flat_idx = (idx + b_off).reshape(B * C)
        zero = (x * 0.0).reshape(B * S, D)
        upd = _scatter_add(zero, flat_idx, y.reshape(B * C, D), axis=0)
        return x + upd.reshape(B, S, D)

    x = A_x
    h = x + _A_ref(_layernorm(x, axis=-1), A_k_cache, A_v_cache, A_wq, A_wo)
    h2 = h + _B_ref(_layernorm(h, axis=-1), B_w_r, B_w_gate, B_w_up, B_w_down)
    return h2
```

```python
import functools

import jax
import jax.numpy as jnp
import jax.experimental.pallas as pl
import jax.experimental.pallas.tpu as pltpu

_EPS = 1e-5
_RB = 64
_NS = 16
_CW = 1024
_PAIRS = (0, 4, 1, 5, 2, 6, 3, 7)
_VISITS = 4
_LAG = 3
_FW = 256


def _layernorm(x):
    m = jnp.mean(x, axis=-1, keepdims=True)
    d = x - m
    v = jnp.mean(d * d, axis=-1, keepdims=True)
    return d / jnp.sqrt(v + _EPS)


def _dot(a, b):
    return jnp.dot(a, b, preferred_element_type=jnp.float32)


def _dot_nt(a, b):
    return jax.lax.dot_general(
        a, b, (((1,), (1,)), ((), ())), preferred_element_type=jnp.float32
    )


def _wait_all(buf, sem):
    pltpu.make_async_copy(buf, buf, sem).wait()


def _loop(lo, hi, body):
    jax.lax.fori_loop(lo, hi, lambda i, carry: body(i), None)


def _ds(start, size):
    return pl.ds(pl.multiple_of(start, size), size)


def _body(
    x_hbm, kt_hbm, vt_hbm, wq_hbm, wo_hbm, wr_hbm, wg_hbm, wu_hbm, wd_hbm,
    out_ref,
    buf, wqbuf, wobuf, wgbuf, wubuf, wdbuf, xbuf, wrbuf,
    q_scr, o_scr, lhs_scr, s_scr, p_scr, l_scr, acc_scr,
    sem, wsem, gsem, dsem,
    *, B, H, Dh, Sk, D, F,
):
    W = _NS * _RB
    NW = H * Dh // W
    HG = 3 * W // Dh
    NC = Sk // _CW
    NF = F // _FW
    steps = (_RB // 8) * NC // _VISITS
    n_groups = B * NW // 3
    scale = Dh ** -0.5

    def issue_cache(src, win, slot, i):
        def visit(u):
            u = i * _VISITS + u
            rows = _ds((u // NC) * 8, 8)
            cols = _ds((u % NC) * _CW, _CW)
            for j, pair in enumerate(_PAIRS):
                pltpu.make_async_copy(
                    src.at[pl.ds(win * _NS + 2 * pair, 2), rows, cols],
                    buf.at[slot, pl.ds(2 * pair, 2), rows, cols],
                    sem.at[slot],
                ).start(priority=j % 2)

        _loop(0, _VISITS, visit)

    def issue_wq(i):
        cw = H * Dh // 3
        n = D // 8 * 3 // 8
        for j in _PAIRS:
            piece = j * n + i
            rows, cols = _ds((piece // 3) * 8, 8), _ds((piece % 3) * cw, cw)
            pltpu.make_async_copy(
                wq_hbm.at[rows, cols], wqbuf.at[rows, cols], wsem.at[2]
            ).start(priority=j // 4)

    def issue_wo(i):
        n = H * Dh // 32 // 8
        for j in _PAIRS:
            rows = _ds((j * n + i) * 32, 32)
            pltpu.make_async_copy(wo_hbm.at[rows, :], wobuf.at[rows, :], wsem.at[3]).start(
                priority=j // 4
            )

    def issue_gate_up(i):
        n = D // 8 // 2
        for j in range(2):
            rows = _ds((j * n + i) * 8, 8)
            pltpu.make_async_copy(wg_hbm.at[rows, :], wgbuf.at[rows, :], gsem.at[0]).start(
                priority=0
            )
            pltpu.make_async_copy(wu_hbm.at[rows, :], wubuf.at[rows, :], gsem.at[1]).start(
                priority=1
            )

    def issue_down(f):
        for j in _PAIRS:
            pltpu.make_async_copy(
                wd_hbm.at[_ds(f * _FW + j * 32, 32), :],
                wdbuf.at[f, pl.ds(j * 32, 32), :],
                dsem.at[f],
            ).start(priority=j // 4)

    def own_head(j):
        lo = jax.lax.broadcasted_iota(jnp.int32, (HG, W), 0) * Dh
        col = jax.lax.broadcasted_iota(jnp.int32, (HG, W), 1) + j * W
        return (lo <= col) & (col < lo + Dh)

    def window(slot, c):
        return buf[slot, pl.ds(0, _NS), pl.ds(0, _RB), _ds(c * _CW, _CW)].reshape(W, _CW)

    def wait_window(slot):
        _wait_all(buf.at[slot, pl.ds(0, _NS), pl.ds(0, _RB), pl.ds(0, Sk)], sem.at[slot])

    def consume_k(win, slot, c):
        @pl.when(c == 0)
        def _():
            wait_window(slot)
            q = q_scr[win % NW, pl.ds(win // NW, 1), :]
            lhs_scr[...] = jnp.where(own_head(win % 3), q, 0.0).astype(lhs_scr.dtype)

        s_scr[:, _ds(c * _CW, _CW)] += _dot(lhs_scr[...], window(slot, c))

    def softmax():
        s = s_scr[...] * scale
        e = jnp.exp(s - jnp.max(s, axis=-1, keepdims=True))
        l_scr[...] = jnp.sum(e, axis=-1, keepdims=True)
        p_scr[...] = e.astype(p_scr.dtype)
        s_scr[...] = jnp.zeros_like(s_scr)

    def consume_v(win, slot, c):
        @pl.when(c == 0)
        def _():
            wait_window(slot)
            acc_scr[...] = jnp.zeros_like(acc_scr)

        acc_scr[...] += _dot_nt(p_scr[:, _ds(c * _CW, _CW)], window(slot, c))

        @pl.when(c == NC - 1)
        def _():
            o = jnp.where(own_head(win % 3), acc_scr[...] / l_scr[...], 0.0)
            o_scr[win % NW, pl.ds(win // NW, 1), :] = jnp.sum(o, axis=0, keepdims=True)

    x_cp = pltpu.make_async_copy(x_hbm, xbuf, wsem.at[0])
    wr_cp = pltpu.make_async_copy(wr_hbm, wrbuf, wsem.at[1])
    x_cp.start()
    wr_cp.start(priority=1)
    _loop(0, D // 8 * 3 // 8, issue_wq)

    x_cp.wait()
    x4 = xbuf[...].astype(jnp.float32)
    x = jnp.concatenate([x4, x4], axis=0)
    xn = _layernorm(x).astype(jnp.bfloat16)
    s_scr[...] = jnp.zeros_like(s_scr)
    o_scr[...] = jnp.zeros_like(o_scr)

    def first_step(i):
        issue_cache(kt_hbm, 0, 0, i)
        pl.when(i == _LAG)(lambda: _wait_all(wqbuf, wsem.at[2]))

        @pl.when((i >= _LAG) & (i < _LAG + NW))
        def _():
            q_scr[i - _LAG] = _dot(xn, wqbuf[:, _ds((i - _LAG) * W, W)])

    _loop(0, steps, first_step)

    def step(n):
        t, i = n // steps, n % steps
        g, j = t // 6, t % 6
        pl.when(j < 3)(lambda: issue_cache(kt_hbm, 3 * g + j, t % 2, i))
        pl.when(j >= 3)(lambda: issue_cache(vt_hbm, 3 * g + j - 3, t % 2, i))
        g, j = (t - 1) // 6, (t - 1) % 6

        @pl.when((i >= _LAG) & (i < _LAG + NC))
        def _():
            pl.when(j < 3)(lambda: consume_k(3 * g + j, (t - 1) % 2, i - _LAG))
            pl.when(j >= 3)(lambda: consume_v(3 * g + j - 3, (t - 1) % 2, i - _LAG))

        pl.when((j == 2) & (i == _LAG + NC))(softmax)

    _loop(steps, 6 * n_groups * steps, step)

    def last_step(i):
        _loop(2 * i, 2 * i + 2, issue_wo)
        pl.when(i >= 4)(lambda: consume_v(B * NW - 1, 1, i - 4))

    _loop(0, 12, last_step)
    _loop(0, 24, issue_gate_up)
    _wait_all(wobuf, wsem.at[3])
    h = x
    for w in range(NW):
        h = h + _dot(o_scr[w].astype(jnp.bfloat16), wobuf[pl.ds(w * W, W), :])
        if w == NW // 2 - 1:
            _loop(24, 40, issue_gate_up)
    _loop(0, NF, issue_down)

    hn = _layernorm(h)
    hb = hn.astype(jnp.bfloat16)
    wr_cp.wait()
    r = jnp.sum(hn * wrbuf[...].astype(jnp.float32).reshape(1, D), axis=-1, keepdims=True)
    _wait_all(wgbuf, gsem.at[0])
    gate = _dot(hb, wgbuf[...])
    _wait_all(wubuf, gsem.at[1])
    act = (gate * jax.nn.sigmoid(gate) * _dot(hb, wubuf[...])).astype(jnp.bfloat16)
    y = jnp.zeros((2 * B, D), jnp.float32)
    for f in range(NF):
        _wait_all(wdbuf.at[f], dsem.at[f])
        y = y + _dot(act[:, f * _FW:(f + 1) * _FW], wdbuf[f])
    y = y * jax.nn.sigmoid(r)
    out = h + (hn + (hn * 0.0 + y))
    out_ref[...] = out[:B].astype(out_ref.dtype)


@jax.jit
def pallas_sequential_preLN__mha_block_cached__moe_arch_mod__decode_kernel(
    A_x: jax.Array,
    A_k_cache: jax.Array,
    A_v_cache: jax.Array,
    A_wq: jax.Array,
    A_wo: jax.Array,
    B_x: jax.Array,
    B_w_r: jax.Array,
    B_w_gate: jax.Array,
    B_w_up: jax.Array,
    B_w_down: jax.Array,
):
    del B_x
    B, Sq, D = A_x.shape
    _, H, Sk, Dh = A_k_cache.shape
    F = B_w_gate.shape[1]
    assert (B, Sq, D, H, Sk, Dh, F) == (4, 1, 640, 32, 8192, 192, 1536)
    W = _NS * _RB
    HG = 3 * W // Dh
    dt = A_k_cache.dtype
    f32 = jnp.float32

    kt = jnp.swapaxes(A_k_cache, 2, 3).reshape(B * H * Dh // _RB, _RB, Sk)
    vt = jnp.swapaxes(A_v_cache, 2, 3).reshape(B * H * Dh // _RB, _RB, Sk)

    out = pl.pallas_call(
        functools.partial(_body, B=B, H=H, Dh=Dh, Sk=Sk, D=D, F=F),
        in_specs=[pl.BlockSpec(memory_space=pl.ANY)] * 9,
        out_specs=pl.BlockSpec(memory_space=pltpu.VMEM),
        out_shape=jax.ShapeDtypeStruct((B, D), A_x.dtype),
        scratch_shapes=[
            pltpu.VMEM((2, _NS, _RB, Sk), dt),
            pltpu.VMEM((D, H * Dh), dt),
            pltpu.VMEM((H * Dh, D), dt),
            pltpu.VMEM((D, F), dt),
            pltpu.VMEM((D, F), dt),
            pltpu.VMEM((F // _FW, _FW, D), dt),
            pltpu.VMEM((B, D), dt),
            pltpu.VMEM((D,), dt),
            pltpu.VMEM((H * Dh // W, 2 * B, W), f32),
            pltpu.VMEM((H * Dh // W, 2 * B, W), f32),
            pltpu.VMEM((HG, W), dt),
            pltpu.VMEM((HG, Sk), f32),
            pltpu.VMEM((HG, Sk), dt),
            pltpu.VMEM((HG, 1), f32),
            pltpu.VMEM((HG, W), f32),
            pltpu.SemaphoreType.DMA((2,)),
            pltpu.SemaphoreType.DMA((4,)),
            pltpu.SemaphoreType.DMA((2,)),
            pltpu.SemaphoreType.DMA((F // _FW,)),
        ],
        compiler_params=pltpu.CompilerParams(vmem_limit_bytes=80 * 1024 * 1024),
    )(A_x.reshape(B, D), kt, vt, A_wq, A_wo, B_w_r, B_w_gate, B_w_up, B_w_down)
    return out.reshape(B, Sq, D)
```

```python
import functools

import jax
import jax.numpy as jnp
import jax.experimental.pallas as pl
import jax.experimental.pallas.tpu as pltpu

_EPS = 1e-5
_RB = 64
_NS = 16
_CW = 1024
_MW = 512
_PAIRS = ((0, 1, 2, 3), (4, 5, 6, 7))
_SKEW = 3
_VISITS = 2
_LAG = 6
_WS = 8
_FW = 256


def _layernorm(x):
    m = jnp.mean(x, axis=-1, keepdims=True)
    d = x - m
    v = jnp.mean(d * d, axis=-1, keepdims=True)
    return d / jnp.sqrt(v + _EPS)


def _dot(a, b):
    return jnp.dot(a, b, preferred_element_type=jnp.float32)


def _dot_nt(a, b):
    return jax.lax.dot_general(
        a, b, (((1,), (1,)), ((), ())), preferred_element_type=jnp.float32
    )


def _wait_all(buf, sem):
    pltpu.make_async_copy(buf, buf, sem).wait()


def _loop(lo, hi, body):
    jax.lax.fori_loop(lo, hi, lambda i, carry: body(i), None)


def _ds(start, size):
    return pl.ds(pl.multiple_of(start, size), size)


def _body(
    x_hbm, kt_hbm, vt_hbm, wq_hbm, wo_hbm, wr_hbm, wg_hbm, wu_hbm, wd_hbm,
    out_ref,
    buf, wqbuf, wobuf, wgbuf, wubuf, wdbuf, xbuf, wrbuf,
    q_scr, o_scr, lhs_scr, s_scr, p_scr, l_scr, acc_scr, h_scr,
    sem, wsem, gsem, dsem,
    *, B, H, Dh, Sk, D, F,
):
    W = _NS * _RB
    NW = H * Dh // W
    HG = 3 * W // Dh
    NC = Sk // _CW
    NM = Sk // _MW
    NF = F // _FW
    steps = (_RB // 8) * NC // _VISITS
    n_cache = 2 * B * NW * steps
    scale = Dh ** -0.5

    def cache_copies(src, win, slot, i, q):
        out = []
        for u in range(_VISITS):
            u = i * _VISITS + u
            rows, cols = _ds((u // NC) * 8, 8), _ds((u % NC) * _CW, _CW)
            for pair in _PAIRS[q]:
                out.append(pltpu.make_async_copy(
                    src.at[pl.ds(win * _NS + 2 * pair, 2), rows, cols],
                    buf.at[slot, pl.ds(2 * pair, 2), rows, cols],
                    sem.at[slot],
                ))
        return out

    def k_copies(n, q):
        t = n // steps
        return cache_copies(kt_hbm, t // 6 * 3 + t % 3, t % 2, n % steps, q)

    def v_copies(n, q):
        t = n // steps
        return cache_copies(vt_hbm, t // 6 * 3 + t % 3, t % 2, n % steps, q)

    def wq_copies(i, q):
        out = []
        for u in range(4):
            u = i * 4 + u
            rows, cols = _ds((u // NW) * 8, 8), _ds((u % NW) * W, W)
            for pair in (2 * q, 2 * q + 1):
                part = (pl.ds(2 * pair, 2), rows, cols)
                out.append(pltpu.make_async_copy(wq_hbm.at[part], wqbuf.at[part], wsem.at[2]))
        return out

    def wo_copies(i, q):
        parts = [(pl.ds(4 * q, 4), _ds((i * 8 + u) * 8, 8)) for u in range(8)]
        return [pltpu.make_async_copy(wo_hbm.at[p], wobuf.at[p], wsem.at[3]) for p in parts]

    def gate_up_copies(i, q):
        src, dst = ((wg_hbm, wgbuf), (wu_hbm, wubuf))[q]
        rows = [_ds((u % 2) * (D // 2) + (i * 4 + u // 2) * 8, 8) for u in range(8)]
        return [pltpu.make_async_copy(src.at[r, :], dst.at[r, :], gsem.at[q]) for r in rows]

    def down_copies(i, q):
        out = []
        for f in range(2):
            f = 2 * i + f
            for j in range(4 * q, 4 * q + 4):
                out.append(pltpu.make_async_copy(
                    wd_hbm.at[_ds(f * _FW + j * 32, 32), :],
                    wdbuf.at[f, pl.ds(j * 32, 32), :],
                    dsem.at[f],
                ))
        return out

    def start(c0, c1):
        for j in range(max(len(c0), len(c1))):
            if c0:
                c0[j].start(priority=0)
            if c1:
                c1[j].start(priority=1)

    def phase(copies, n, after, work=lambda i: None):
        _loop(0, n - _SKEW, lambda i: (start(copies(i, 0), copies(i + _SKEW, 1)), work(i))[0])
        _loop(n - _SKEW, n, lambda i: (start(copies(i, 0), after(i + _SKEW - n, 1)), work(i))[0])

    def wo_flat(w):
        return wobuf.reshape(H * Dh, D)[_ds(w * W, W), :]

    def own_head(j):
        lo = jax.lax.broadcasted_iota(jnp.int32, (HG, W), 0) * Dh
        col = jax.lax.broadcasted_iota(jnp.int32, (HG, W), 1) + j * W
        return (lo <= col) & (col < lo + Dh)

    def window(slot, c):
        return buf[slot, pl.ds(0, _NS), pl.ds(0, _RB), _ds(c * _MW, _MW)].reshape(W, _MW)

    def wait_window(slot):
        _wait_all(buf.at[slot, pl.ds(0, _NS), pl.ds(0, _RB), pl.ds(0, Sk)], sem.at[slot])

    def consume_k(win, slot, c):
        @pl.when(c == 0)
        def _():
            wait_window(slot)
            q = q_scr[win % NW, pl.ds(win // NW, 1), :]
            lhs_scr[...] = jnp.where(own_head(win % 3), q, 0.0).astype(lhs_scr.dtype)

        s_scr[:, _ds(c * _MW, _MW)] += _dot(lhs_scr[...], window(slot, c))

    def softmax():
        s = s_scr[...] * scale
        e = jnp.exp(s - jnp.max(s, axis=-1, keepdims=True))
        l_scr[...] = jnp.sum(e, axis=-1, keepdims=True)
        p_scr[...] = e.astype(p_scr.dtype)
        s_scr[...] = jnp.zeros_like(s_scr)

    def consume_v(win, slot, c):
        @pl.when(c == 0)
        def _():
            wait_window(slot)
            acc_scr[...] = jnp.zeros_like(acc_scr)

        acc_scr[...] += _dot_nt(p_scr[:, _ds(c * _MW, _MW)], window(slot, c))

        @pl.when(c == NM - 1)
        def _():
            o = jnp.where(own_head(win % 3), acc_scr[...] / l_scr[...], 0.0)
            o_scr[win % NW, pl.ds(win // NW, 1), :] = jnp.sum(o, axis=0, keepdims=True)

    x_cp = pltpu.make_async_copy(x_hbm, xbuf, wsem.at[0])
    wr_cp = pltpu.make_async_copy(wr_hbm, wrbuf, wsem.at[1])
    _loop(0, _SKEW, lambda i: start([], wq_copies(i, 1)))
    x_cp.start()
    wr_cp.start()
    phase(wq_copies, D // _WS // 8 * NW // 4, k_copies)

    x_cp.wait()
    x4 = xbuf[...].astype(jnp.float32)
    x = jnp.concatenate([x4, x4], axis=0)
    xn = _layernorm(x).astype(jnp.bfloat16)
    s_scr[...] = jnp.zeros_like(s_scr)
    o_scr[...] = jnp.zeros_like(o_scr)

    def project(i):
        pl.when(i == _LAG)(lambda: _wait_all(wqbuf, wsem.at[2]))

        @pl.when((i >= _LAG) & (i < _LAG + NW))
        def _():
            q_scr[i - _LAG] = _dot(xn, wqbuf[:, :, _ds((i - _LAG) * W, W)].reshape(D, W))

    _loop(0, steps, lambda i: (start(k_copies(i, 0), k_copies(i + _SKEW, 1)), project(i))[0])

    def step(n):
        m = n + _SKEW
        n_is_k, m_is_k = n // steps % 6 < 3, m // steps % 6 < 3
        last = m >= n_cache
        pl.when(n_is_k & m_is_k)(lambda: start(k_copies(n, 0), k_copies(m, 1)))
        pl.when(n_is_k & ~m_is_k)(lambda: start(k_copies(n, 0), v_copies(m, 1)))
        pl.when(~n_is_k & ~m_is_k)(lambda: start(v_copies(n, 0), v_copies(m, 1)))
        pl.when(~n_is_k & m_is_k & ~last)(lambda: start(v_copies(n, 0), k_copies(m, 1)))
        pl.when(last)(lambda: start(v_copies(n, 0), wo_copies(m - n_cache, 1)))
        t, i = n // steps - 1, n % steps
        win = t // 6 * 3 + t % 3

        @pl.when((i >= _LAG) & (i < _LAG + NM))
        def _():
            pl.when(t % 6 < 3)(lambda: consume_k(win, t % 2, i - _LAG))
            pl.when(t % 6 >= 3)(lambda: consume_v(win, t % 2, i - _LAG))

        pl.when((t % 6 == 2) & (i == _LAG + NM))(softmax)

    _loop(steps, n_cache, step)

    def last_window(lo, hi):
        _loop(lo, hi, lambda c: consume_v(B * NW - 1, 1, c))

    phase(wo_copies, 12, gate_up_copies,
          lambda i: pl.when(i >= 5)(lambda: last_window(2 * (i - 5), 2 * (i - 5) + 2)))
    h_scr[...] = x

    def out_project(i):
        pl.when(i < 2)(lambda: last_window(14 + i, 15 + i))
        pl.when(i == 4)(lambda: _wait_all(wobuf, wsem.at[3]))

        @pl.when(i >= 4)
        def _():
            w = i - 4
            h_scr[...] += _dot(o_scr[w].astype(jnp.bfloat16), wo_flat(w))

    phase(gate_up_copies, 10, down_copies, out_project)
    _loop(0, _SKEW, lambda i: start(down_copies(i, 0), []))
    h = h_scr[...]

    hn = _layernorm(h)
    hb = hn.astype(jnp.bfloat16)
    wr_cp.wait()
    r = jnp.sum(hn * wrbuf[...].astype(jnp.float32).reshape(1, D), axis=-1, keepdims=True)
    _wait_all(wgbuf, gsem.at[0])
    gate = _dot(hb, wgbuf[...])
    _wait_all(wubuf, gsem.at[1])
    act = (gate * jax.nn.sigmoid(gate) * _dot(hb, wubuf[...])).astype(jnp.bfloat16)
    y = jnp.zeros((2 * B, D), jnp.float32)
    for f in range(NF):
        _wait_all(wdbuf.at[f], dsem.at[f])
        y = y + _dot(act[:, f * _FW:(f + 1) * _FW], wdbuf[f])
    y = y * jax.nn.sigmoid(r)
    out = h + (hn + (hn * 0.0 + y))
    out_ref[...] = out[:B].astype(out_ref.dtype)


@jax.jit
def pallas_sequential_preLN__mha_block_cached__moe_arch_mod__decode_kernel(
    A_x: jax.Array,
    A_k_cache: jax.Array,
    A_v_cache: jax.Array,
    A_wq: jax.Array,
    A_wo: jax.Array,
    B_x: jax.Array,
    B_w_r: jax.Array,
    B_w_gate: jax.Array,
    B_w_up: jax.Array,
    B_w_down: jax.Array,
):
    del B_x
    B, Sq, D = A_x.shape
    _, H, Sk, Dh = A_k_cache.shape
    F = B_w_gate.shape[1]
    assert (B, Sq, D, H, Sk, Dh, F) == (4, 1, 640, 32, 8192, 192, 1536)
    W = _NS * _RB
    HG = 3 * W // Dh
    dt = A_k_cache.dtype
    f32 = jnp.float32

    kt = jnp.swapaxes(A_k_cache, 2, 3).reshape(B * H * Dh // _RB, _RB, Sk)
    vt = jnp.swapaxes(A_v_cache, 2, 3).reshape(B * H * Dh // _RB, _RB, Sk)

    wq = A_wq.reshape(_WS, D // _WS, H * Dh)
    wo = A_wo.reshape(_WS, H * Dh // _WS, D)

    out = pl.pallas_call(
        functools.partial(_body, B=B, H=H, Dh=Dh, Sk=Sk, D=D, F=F),
        in_specs=[pl.BlockSpec(memory_space=pl.ANY)] * 9,
        out_specs=pl.BlockSpec(memory_space=pltpu.VMEM),
        out_shape=jax.ShapeDtypeStruct((B, D), A_x.dtype),
        scratch_shapes=[
            pltpu.VMEM((2, _NS, _RB, Sk), dt),
            pltpu.VMEM((_WS, D // _WS, H * Dh), dt),
            pltpu.VMEM((_WS, H * Dh // _WS, D), dt),
            pltpu.VMEM((D, F), dt),
            pltpu.VMEM((D, F), dt),
            pltpu.VMEM((F // _FW, _FW, D), dt),
            pltpu.VMEM((B, D), dt),
            pltpu.VMEM((D,), dt),
            pltpu.VMEM((H * Dh // W, 2 * B, W), f32),
            pltpu.VMEM((H * Dh // W, 2 * B, W), f32),
            pltpu.VMEM((HG, W), dt),
            pltpu.VMEM((HG, Sk), f32),
            pltpu.VMEM((HG, Sk), dt),
            pltpu.VMEM((HG, 1), f32),
            pltpu.VMEM((HG, W), f32),
            pltpu.VMEM((2 * B, D), f32),
            pltpu.SemaphoreType.DMA((2,)),
            pltpu.SemaphoreType.DMA((4,)),
            pltpu.SemaphoreType.DMA((2,)),
            pltpu.SemaphoreType.DMA((F // _FW,)),
        ],
        compiler_params=pltpu.CompilerParams(
            vmem_limit_bytes=80 * 1024 * 1024, disable_bounds_checks=True
        ),
    )(A_x.reshape(B, D), kt, vt, wq, wo, B_w_r, B_w_gate, B_w_up, B_w_down)
    return out.reshape(B, Sq, D)
```

```python
import functools

import jax
import jax.numpy as jnp
import jax.experimental.pallas as pl
import jax.experimental.pallas.tpu as pltpu

_EPS = 1e-5
_RB = 64
_NS = 16
_CW = 1024
_MW = 512
_PAIRS = ((0, 2, 4, 6), (1, 3, 5, 7))
_SKEW = 26
_VISITS = 2
_LAG = 6
_WS = 8
_DS = 4
_DP = 128


def _layernorm(x):
    m = jnp.mean(x, axis=-1, keepdims=True)
    d = x - m
    v = jnp.mean(d * d, axis=-1, keepdims=True)
    return d / jnp.sqrt(v + _EPS)


def _dot(a, b):
    return jnp.dot(a, b, preferred_element_type=jnp.float32)


def _dot_nt(a, b):
    return jax.lax.dot_general(
        a, b, (((1,), (1,)), ((), ())), preferred_element_type=jnp.float32
    )


def _wait_all(buf, sem):
    pltpu.make_async_copy(buf, buf, sem).wait()


def _loop(lo, hi, body):
    jax.lax.fori_loop(lo, hi, lambda i, carry: body(i), None)


def _ds(start, size):
    return pl.ds(pl.multiple_of(start, size), size)


def _body(
    x_hbm, kt_hbm, vt_hbm, wq_hbm, wo_hbm, wr_hbm, wg_hbm, wu_hbm, wd_hbm,
    out_ref,
    buf, wqbuf, wobuf, wgbuf, wubuf, wdbuf, xbuf, wrbuf,
    q_scr, o_scr, lhs_scr, s_scr, p_scr, l_scr, acc_scr, h_scr,
    sem, wsem, gsem, dsem,
    *, B, H, Dh, Sk, D, F,
):
    W = _NS * _RB
    NW = H * Dh // W
    HG = 3 * W // Dh
    NC = Sk // _CW
    NM = Sk // _MW
    steps = (_RB // 8) * NC // _VISITS
    n_groups = B * NW // 3
    sk, rem = divmod(_SKEW, 8)
    scale = Dh ** -0.5

    def cache_copies(src, g, first_slot, n, q):
        win, slot, i = 3 * g + n // steps, (first_slot + n // steps) % 2, n % steps
        out = []
        for u in range(_VISITS):
            u = i * _VISITS + u
            rows, cols = _ds((u // NC) * 8, 8), _ds((u % NC) * _CW, _CW)
            for pair in _PAIRS[q]:
                out.append(pltpu.make_async_copy(
                    src.at[pl.ds(win * _NS + 2 * pair, 2), rows, cols],
                    buf.at[slot, pl.ds(2 * pair, 2), rows, cols],
                    sem.at[slot],
                ))
        return out

    def wq_copies(i, q):
        out = []
        for u in range(4):
            u = i * 4 + u
            rows, cols = _ds((u // NW) * 8, 8), _ds((u % NW) * W, W)
            for pair in (2 * q, 2 * q + 1):
                part = (pl.ds(2 * pair, 2), rows, cols)
                out.append(pltpu.make_async_copy(wq_hbm.at[part], wqbuf.at[part], wsem.at[2]))
        return out

    def wo_copies(i, q):
        parts = [(pl.ds(4 * q, 4), _ds((i * 8 + u) * 8, 8)) for u in range(8)]
        return [pltpu.make_async_copy(wo_hbm.at[p], wobuf.at[p], wsem.at[3]) for p in parts]

    def gate_up_copies(i, q):
        src, dst = ((wg_hbm, wgbuf), (wu_hbm, wubuf))[q]
        rows = [_ds((u % 2) * (D // 2) + (i * 4 + u // 2) * 8, 8) for u in range(8)]
        return [pltpu.make_async_copy(src.at[r, :], dst.at[r, :], gsem.at[q]) for r in rows]

    def down_copies(q):
        n = _DS // 2
        out = []
        for lo in range(0, F // _DS, 32 // n):
            part = (pl.ds(n * q, n), pl.ds(lo, 32 // n))
            out.append(pltpu.make_async_copy(wd_hbm.at[part], wdbuf.at[part], dsem.at[lo // _DP]))
        return out

    def start(c0, c1):
        for j in range(max(len(c0), len(c1))):
            if j < len(c0):
                c0[j].start(priority=0)
            if j < len(c1):
                c1[j].start(priority=1)

    def ahead(first, second, i):
        return first(i + sk, 1)[rem:] + second(i + sk + 1, 1)[:rem]

    def phase(copies, n, after, work=lambda i: None, late_work=lambda i: None):
        nxt = lambda i, q: after(i - n, q)
        mid = n - sk - 1
        _loop(0, mid, lambda i: (start(copies(i, 0), ahead(copies, copies, i)), work(i))[0])
        _loop(mid, mid + 1, lambda i: (start(copies(i, 0), ahead(copies, nxt, i)), late_work(i))[0])
        _loop(mid + 1, n, lambda i: (start(copies(i, 0), ahead(nxt, nxt, i)), late_work(i))[0])

    def own_head(j):
        lo = jax.lax.broadcasted_iota(jnp.int32, (HG, W), 0) * Dh
        col = jax.lax.broadcasted_iota(jnp.int32, (HG, W), 1) + j * W
        return (lo <= col) & (col < lo + Dh)

    def window(slot, c):
        return buf[slot, pl.ds(0, _NS), pl.ds(0, _RB), _ds(c * _MW, _MW)].reshape(W, _MW)

    def wait_window(slot):
        _wait_all(buf.at[slot, pl.ds(0, _NS), pl.ds(0, _RB), pl.ds(0, Sk)], sem.at[slot])

    def consume_k(win, slot, c):
        @pl.when(c == 0)
        def _():
            wait_window(slot)
            q = q_scr[win % NW, pl.ds(win // NW, 1), :]
            lhs_scr[...] = jnp.where(own_head(win % 3), q, 0.0).astype(lhs_scr.dtype)

        s_scr[:, _ds(c * _MW, _MW)] += _dot(lhs_scr[...], window(slot, c))

    def softmax():
        s = s_scr[...] * scale
        e = jnp.exp(s - jnp.max(s, axis=-1, keepdims=True))
        l_scr[...] = jnp.sum(e, axis=-1, keepdims=True)
        p_scr[...] = e.astype(p_scr.dtype)
        s_scr[...] = jnp.zeros_like(s_scr)

    def consume_v(win, slot, c):
        @pl.when(c == 0)
        def _():
            wait_window(slot)
            acc_scr[...] = jnp.zeros_like(acc_scr)

        acc_scr[...] += _dot_nt(p_scr[:, _ds(c * _MW, _MW)], window(slot, c))

        @pl.when(c == NM - 1)
        def _():
            o = jnp.where(own_head(win % 3), acc_scr[...] / l_scr[...], 0.0)
            o_scr[win % NW, pl.ds(win // NW, 1), :] = jnp.sum(o, axis=0, keepdims=True)

    x_cp = pltpu.make_async_copy(x_hbm, xbuf, wsem.at[0])
    wr_cp = pltpu.make_async_copy(wr_hbm, wrbuf, wsem.at[1])
    k_copies = lambda g: functools.partial(cache_copies, kt_hbm, g, 0)
    v_copies = lambda g: functools.partial(cache_copies, vt_hbm, g, 1)
    _loop(0, sk, lambda i: start([], wq_copies(i, 1)))
    _loop(sk, sk + 1, lambda i: start([], wq_copies(i, 1)[:rem]))
    x_cp.start()
    wr_cp.start()
    phase(wq_copies, D // _WS // 8 * NW // 4, k_copies(0))

    x_cp.wait()
    x4 = xbuf[...].astype(jnp.float32)
    x = jnp.concatenate([x4, x4], axis=0)
    xn = _layernorm(x).astype(jnp.bfloat16)
    s_scr[...] = jnp.zeros_like(s_scr)
    o_scr[...] = jnp.zeros_like(o_scr)

    def project(i):
        pl.when(i == _LAG)(lambda: _wait_all(wqbuf, wsem.at[2]))

        @pl.when((i >= _LAG) & (i < _LAG + NW))
        def _():
            q_scr[i - _LAG] = _dot(xn, wqbuf[:, :, _ds((i - _LAG) * W, W)].reshape(D, W))

    def head_group(g):
        def during_k(n):
            j, i = n // steps, n % steps
            pl.when((g == 0) & (j == 0))(lambda: project(i))

            @pl.when((i >= _LAG) & (i < _LAG + NM))
            def _():
                pl.when((j == 0) & (g > 0))(lambda: consume_v(3 * g - 1, 1, i - _LAG))
                pl.when(j > 0)(lambda: consume_k(3 * g + j - 1, (j - 1) % 2, i - _LAG))

        def during_v(n):
            j, i = n // steps, n % steps

            @pl.when((i >= _LAG) & (i < _LAG + NM))
            def _():
                pl.when(j == 0)(lambda: consume_k(3 * g + 2, 0, i - _LAG))
                pl.when(j > 0)(lambda: consume_v(3 * g + j - 1, j % 2, i - _LAG))

            pl.when((j == 0) & (i == _LAG + NM))(softmax)

        phase(k_copies(g), 3 * steps, v_copies(g), during_k)
        return during_v

    def full_group(g):
        phase(v_copies(g), 3 * steps, k_copies(g + 1), head_group(g))

    _loop(0, n_groups - 1, full_group)
    _loop(n_groups - 1, n_groups, lambda g: phase(v_copies(g), 3 * steps, wo_copies, head_group(g)))

    def last_window(lo, hi):
        _loop(lo, hi, lambda c: consume_v(B * NW - 1, 1, c))

    def during_wo(i):
        pl.when(i >= 4)(lambda: last_window(2 * (i - 4), 2 * (i - 4) + 2))

    phase(wo_copies, 12, gate_up_copies, during_wo, during_wo)
    h_scr[...] = x

    def out_project(i):
        pl.when(i == 4)(lambda: _wait_all(wobuf, wsem.at[3]))

        @pl.when(i >= 4)
        def _():
            w = 2 * (i - 4)
            o = jnp.concatenate([o_scr[w], o_scr[w + 1]], axis=1).astype(jnp.bfloat16)
            h_scr[...] += _dot(o, wobuf.reshape(H * Dh, D)[_ds(w * W, 2 * W), :])

    gu = gate_up_copies
    down = down_copies(1)
    _loop(0, 9 - sk, lambda i: (start(gu(i, 0), ahead(gu, gu, i)), out_project(i))[0])
    _loop(9 - sk, 10 - sk, lambda i: (start(gu(i, 0), gu(i + sk, 1)[rem:] + down[:rem]), out_project(i))[0])
    h = h_scr[...]
    hn = _layernorm(h)
    hb = hn.astype(jnp.bfloat16)
    wr_cp.wait()
    r = jnp.sum(hn * wrbuf[...].astype(jnp.float32).reshape(1, D), axis=-1, keepdims=True)
    route = jax.nn.sigmoid(r)
    for j, i in enumerate(range(10 - sk, 10)):
        _loop(i, i + 1, lambda i: start(gu(i, 0), down[rem + 8 * j:rem + 8 * j + 8]))
    start(down_copies(0), [])

    _wait_all(wgbuf, gsem.at[0])
    _wait_all(wubuf, gsem.at[1])
    gate = _dot(hb, wgbuf[...])
    act = (gate * jax.nn.sigmoid(gate) * _dot(hb, wubuf[...])).astype(jnp.bfloat16)
    y = jnp.zeros((2 * B, D), jnp.float32)
    for lo in range(0, F // _DS, _DP):
        piece = wdbuf.at[:, pl.ds(lo, _DP), :]
        _wait_all(piece, dsem.at[lo // _DP])
        a = jnp.concatenate([act[:, c + lo:c + lo + _DP] for c in range(0, F, F // _DS)], axis=1)
        y = y + _dot(a, piece[...].reshape(_DS * _DP, D))
    out = h + (hn + (hn * 0.0 + y * route))
    out_ref[...] = out[:B].astype(out_ref.dtype)


@jax.jit
def pallas_sequential_preLN__mha_block_cached__moe_arch_mod__decode_kernel(
    A_x: jax.Array,
    A_k_cache: jax.Array,
    A_v_cache: jax.Array,
    A_wq: jax.Array,
    A_wo: jax.Array,
    B_x: jax.Array,
    B_w_r: jax.Array,
    B_w_gate: jax.Array,
    B_w_up: jax.Array,
    B_w_down: jax.Array,
):
    del B_x
    B, Sq, D = A_x.shape
    _, H, Sk, Dh = A_k_cache.shape
    F = B_w_gate.shape[1]
    assert (B, Sq, D, H, Sk, Dh, F) == (4, 1, 640, 32, 8192, 192, 1536)
    W = _NS * _RB
    HG = 3 * W // Dh
    dt = A_k_cache.dtype
    f32 = jnp.float32

    kt = jnp.swapaxes(A_k_cache, 2, 3).reshape(B * H * Dh // _RB, _RB, Sk)
    vt = jnp.swapaxes(A_v_cache, 2, 3).reshape(B * H * Dh // _RB, _RB, Sk)

    wq = A_wq.reshape(_WS, D // _WS, H * Dh)
    wo = A_wo.reshape(_WS, H * Dh // _WS, D)
    wd = B_w_down.reshape(_DS, F // _DS, D)

    out = pl.pallas_call(
        functools.partial(_body, B=B, H=H, Dh=Dh, Sk=Sk, D=D, F=F),
        in_specs=[pl.BlockSpec(memory_space=pl.ANY)] * 9,
        out_specs=pl.BlockSpec(memory_space=pltpu.VMEM),
        out_shape=jax.ShapeDtypeStruct((B, D), A_x.dtype),
        scratch_shapes=[
            pltpu.VMEM((2, _NS, _RB, Sk), dt),
            pltpu.VMEM((_WS, D // _WS, H * Dh), dt),
            pltpu.VMEM((_WS, H * Dh // _WS, D), dt),
            pltpu.VMEM((D, F), dt),
            pltpu.VMEM((D, F), dt),
            pltpu.VMEM((_DS, F // _DS, D), dt),
            pltpu.VMEM((B, D), dt),
            pltpu.VMEM((D,), dt),
            pltpu.VMEM((H * Dh // W, 2 * B, W), f32),
            pltpu.VMEM((H * Dh // W, 2 * B, W), f32),
            pltpu.VMEM((HG, W), dt),
            pltpu.VMEM((HG, Sk), f32),
            pltpu.VMEM((HG, Sk), dt),
            pltpu.VMEM((HG, 1), f32),
            pltpu.VMEM((HG, W), f32),
            pltpu.VMEM((2 * B, D), f32),
            pltpu.SemaphoreType.DMA((2,)),
            pltpu.SemaphoreType.DMA((4,)),
            pltpu.SemaphoreType.DMA((2,)),
            pltpu.SemaphoreType.DMA((F // (_DS * _DP),)),
        ],
        compiler_params=pltpu.CompilerParams(
            vmem_limit_bytes=80 * 1024 * 1024, disable_bounds_checks=True
        ),
    )(A_x.reshape(B, D), kt, vt, wq, wo, B_w_r, B_w_gate, B_w_up, wd)
    return out.reshape(B, Sq, D)
```

```python
import functools

import jax
import jax.numpy as jnp
import jax.experimental.pallas as pl
import jax.experimental.pallas.tpu as pltpu

_EPS = 1e-5
_RB = 64
_NS = 16
_CW = 1024
_MW = 512
_PAIRS = ((0, 2, 4, 6), (1, 3, 5, 7))
_SKEW = 26
_VISITS = 2
_LAG = 6
_WS = 8
_DS = 2
_DP = (256, 512, 768)


def _layernorm(x):
    m = jnp.mean(x, axis=-1, keepdims=True)
    d = x - m
    v = jnp.mean(d * d, axis=-1, keepdims=True)
    return d / jnp.sqrt(v + _EPS)


def _dot(a, b):
    return jnp.dot(a, b, preferred_element_type=jnp.float32)


def _dot_nt(a, b):
    return jax.lax.dot_general(
        a, b, (((1,), (1,)), ((), ())), preferred_element_type=jnp.float32
    )


def _wait_all(buf, sem):
    pltpu.make_async_copy(buf, buf, sem).wait()


def _loop(lo, hi, body):
    jax.lax.fori_loop(lo, hi, lambda i, carry: body(i), None)


def _ds(start, size):
    return pl.ds(pl.multiple_of(start, size), size)


def _body(
    x_hbm, kt_hbm, vt_hbm, wq_hbm, wo_hbm, wr_hbm, wg_hbm, wu_hbm, wd_hbm,
    out_ref,
    buf, wqbuf, wobuf, wgbuf, wubuf, wdbuf, xbuf, wrbuf,
    q_scr, o_scr, lhs_scr, s_scr, p_scr, l_scr, acc_scr, h_scr,
    sem, wsem, gsem, dsem,
    *, B, H, Dh, Sk, D, F,
):
    W = _NS * _RB
    NW = H * Dh // W
    HG = 3 * W // Dh
    NC = Sk // _CW
    NM = Sk // _MW
    steps = (_RB // 8) * NC // _VISITS
    n_groups = B * NW // 3
    sk, rem = divmod(_SKEW, 8)
    scale = Dh ** -0.5

    def cache_copies(src, g, first_slot, n, q):
        win, slot, i = 3 * g + n // steps, (first_slot + n // steps) % 2, n % steps
        out = []
        for u in range(_VISITS):
            u = i * _VISITS + u
            rows, cols = _ds((u // NC) * 8, 8), _ds((u % NC) * _CW, _CW)
            for pair in _PAIRS[q]:
                out.append(pltpu.make_async_copy(
                    src.at[pl.ds(win * _NS + 2 * pair, 2), rows, cols],
                    buf.at[slot, pl.ds(2 * pair, 2), rows, cols],
                    sem.at[slot],
                ))
        return out

    def wq_copies(i, q):
        out = []
        for u in range(4):
            u = i * 4 + u
            rows, cols = _ds((u // NW) * 8, 8), _ds((u % NW) * W, W)
            for pair in (2 * q, 2 * q + 1):
                part = (pl.ds(2 * pair, 2), rows, cols)
                out.append(pltpu.make_async_copy(wq_hbm.at[part], wqbuf.at[part], wsem.at[2]))
        return out

    def wo_copies(i, q):
        parts = [(pl.ds(4 * q, 4), _ds((i * 8 + u) * 8, 8)) for u in range(8)]
        return [pltpu.make_async_copy(wo_hbm.at[p], wobuf.at[p], wsem.at[3]) for p in parts]

    def gate_up_copies(i, q):
        src, dst = ((wg_hbm, wgbuf), (wu_hbm, wubuf))[q]
        rows = [_ds((u % 2) * (D // 2) + (i * 4 + u // 2) * 8, 8) for u in range(8)]
        return [pltpu.make_async_copy(src.at[r, :], dst.at[r, :], gsem.at[q]) for r in rows]

    def down_copies(q):
        n = _DS // 2
        out = []
        for lo in range(0, F // _DS, 32 // n):
            part = (pl.ds(n * q, n), pl.ds(lo, 32 // n))
            piece = sum(lo >= end for end in _DP)
            out.append(pltpu.make_async_copy(wd_hbm.at[part], wdbuf.at[part], dsem.at[piece]))
        return out

    def start(c0, c1):
        for j in range(max(len(c0), len(c1))):
            if j < len(c0):
                c0[j].start(priority=0)
            if j < len(c1):
                c1[j].start(priority=1)

    def ahead(first, second, i):
        return first(i + sk, 1)[rem:] + second(i + sk + 1, 1)[:rem]

    def phase(copies, n, after, work=lambda i: None, late_work=lambda i: None):
        nxt = lambda i, q: after(i - n, q)
        mid = n - sk - 1
        _loop(0, mid, lambda i: (start(copies(i, 0), ahead(copies, copies, i)), work(i))[0])
        _loop(mid, mid + 1, lambda i: (start(copies(i, 0), ahead(copies, nxt, i)), late_work(i))[0])
        _loop(mid + 1, n, lambda i: (start(copies(i, 0), ahead(nxt, nxt, i)), late_work(i))[0])

    def own_head(j):
        lo = jax.lax.broadcasted_iota(jnp.int32, (HG, W), 0) * Dh
        col = jax.lax.broadcasted_iota(jnp.int32, (HG, W), 1) + j * W
        return (lo <= col) & (col < lo + Dh)

    def window(slot, c):
        return buf[slot, pl.ds(0, _NS), pl.ds(0, _RB), _ds(c * _MW, _MW)].reshape(W, _MW)

    def wait_window(slot):
        _wait_all(buf.at[slot, pl.ds(0, _NS), pl.ds(0, _RB), pl.ds(0, Sk)], sem.at[slot])

    def consume_k(win, slot, c):
        @pl.when(c == 0)
        def _():
            wait_window(slot)
            q = q_scr[win % NW, pl.ds(win // NW, 1), :]
            lhs_scr[...] = jnp.where(own_head(win % 3), q, 0.0).astype(lhs_scr.dtype)

        s_scr[:, _ds(c * _MW, _MW)] += _dot(lhs_scr[...], window(slot, c))

    def softmax():
        s = s_scr[...] * scale
        e = jnp.exp(s - jnp.max(s, axis=-1, keepdims=True))
        l_scr[...] = jnp.sum(e, axis=-1, keepdims=True)
        p_scr[...] = e.astype(p_scr.dtype)
        s_scr[...] = jnp.zeros_like(s_scr)

    def consume_v(win, slot, c):
        @pl.when(c == 0)
        def _():
            wait_window(slot)
            acc_scr[...] = jnp.zeros_like(acc_scr)

        acc_scr[...] += _dot_nt(p_scr[:, _ds(c * _MW, _MW)], window(slot, c))

        @pl.when(c == NM - 1)
        def _():
            o = jnp.where(own_head(win % 3), acc_scr[...] / l_scr[...], 0.0)
            o_scr[win % NW, pl.ds(win // NW, 1), :] = jnp.sum(o, axis=0, keepdims=True)

    x_cp = pltpu.make_async_copy(x_hbm, xbuf, wsem.at[0])
    wr_cp = pltpu.make_async_copy(wr_hbm, wrbuf, wsem.at[1])
    k_copies = lambda g: functools.partial(cache_copies, kt_hbm, g, 0)
    v_copies = lambda g: functools.partial(cache_copies, vt_hbm, g, 1)
    _loop(0, sk, lambda i: start([], wq_copies(i, 1)))
    _loop(sk, sk + 1, lambda i: start([], wq_copies(i, 1)[:rem]))
    x_cp.start()
    wr_cp.start()
    phase(wq_copies, D // _WS // 8 * NW // 4, k_copies(0))

    x_cp.wait()
    x4 = xbuf[...].astype(jnp.float32)
    x = jnp.concatenate([x4, x4], axis=0)
    xn = _layernorm(x).astype(jnp.bfloat16)
    s_scr[...] = jnp.zeros_like(s_scr)
    o_scr[...] = jnp.zeros_like(o_scr)

    def project(i):
        pl.when(i == _LAG)(lambda: _wait_all(wqbuf, wsem.at[2]))

        @pl.when((i >= _LAG) & (i < _LAG + NW))
        def _():
            q_scr[i - _LAG] = _dot(xn, wqbuf[:, :, _ds((i - _LAG) * W, W)].reshape(D, W))

    def head_group(g):
        def during_k(n):
            j, i = n // steps, n % steps
            pl.when((g == 0) & (j == 0))(lambda: project(i))

            @pl.when((i >= _LAG) & (i < _LAG + NM))
            def _():
                pl.when((j == 0) & (g > 0))(lambda: consume_v(3 * g - 1, 1, i - _LAG))
                pl.when(j > 0)(lambda: consume_k(3 * g + j - 1, (j - 1) % 2, i - _LAG))

        def during_v(n):
            j, i = n // steps, n % steps

            @pl.when((i >= _LAG) & (i < _LAG + NM))
            def _():
                pl.when(j == 0)(lambda: consume_k(3 * g + 2, 0, i - _LAG))
                pl.when(j > 0)(lambda: consume_v(3 * g + j - 1, j % 2, i - _LAG))

            pl.when((j == 0) & (i == _LAG + NM))(softmax)

        phase(k_copies(g), 3 * steps, v_copies(g), during_k)
        return during_v

    def full_group(g):
        phase(v_copies(g), 3 * steps, k_copies(g + 1), head_group(g))

    _loop(0, n_groups - 1, full_group)
    _loop(n_groups - 1, n_groups, lambda g: phase(v_copies(g), 3 * steps, wo_copies, head_group(g)))

    def last_window(lo, hi):
        _loop(lo, hi, lambda c: consume_v(B * NW - 1, 1, c))

    def during_wo(i):
        pl.when(i >= 4)(lambda: last_window(2 * (i - 4), 2 * (i - 4) + 2))

    phase(wo_copies, 12, gate_up_copies, during_wo, during_wo)
    h_scr[...] = x

    def out_project(i):
        pl.when(i == 4)(lambda: _wait_all(wobuf, wsem.at[3]))

        @pl.when(i >= 4)
        def _():
            w = 2 * (i - 4)
            o = jnp.concatenate([o_scr[w], o_scr[w + 1]], axis=1).astype(jnp.bfloat16)
            h_scr[...] += _dot(o, wobuf.reshape(H * Dh, D)[_ds(w * W, 2 * W), :])

    gu = gate_up_copies
    down = down_copies(1)
    _loop(0, 9 - sk, lambda i: (start(gu(i, 0), ahead(gu, gu, i)), out_project(i))[0])
    _loop(9 - sk, 10 - sk, lambda i: (start(gu(i, 0), gu(i + sk, 1)[rem:] + down[:rem]), out_project(i))[0])
    h = h_scr[...]
    hn = _layernorm(h)
    hb = hn.astype(jnp.bfloat16)
    wr_cp.wait()
    r = jnp.sum(hn * wrbuf[...].astype(jnp.float32).reshape(1, D), axis=-1, keepdims=True)
    route = jax.nn.sigmoid(r)
    for j, i in enumerate(range(10 - sk, 10)):
        _loop(i, i + 1, lambda i: start(gu(i, 0), down[rem + 8 * j:rem + 8 * j + 8]))
    start(down_copies(0), [])

    _wait_all(wgbuf, gsem.at[0])
    _wait_all(wubuf, gsem.at[1])
    gate = _dot(hb, wgbuf[...])
    act = (gate * jax.nn.sigmoid(gate) * _dot(hb, wubuf[...])).astype(jnp.bfloat16)
    y = jnp.zeros((2 * B, D), jnp.float32)
    for i, (lo, hi) in enumerate(zip((0,) + _DP, _DP)):
        piece = wdbuf.at[:, pl.ds(lo, hi - lo), :]
        a = jnp.concatenate([act[:, c + lo:c + hi] for c in range(0, F, F // _DS)], axis=1)
        _wait_all(piece, dsem.at[i])
        y = y + _dot(a, piece[...].reshape(_DS * (hi - lo), D))
    out = h + (hn + (hn * 0.0 + y * route))
    out_ref[...] = out[:B].astype(out_ref.dtype)


@jax.jit
def pallas_sequential_preLN__mha_block_cached__moe_arch_mod__decode_kernel(
    A_x: jax.Array,
    A_k_cache: jax.Array,
    A_v_cache: jax.Array,
    A_wq: jax.Array,
    A_wo: jax.Array,
    B_x: jax.Array,
    B_w_r: jax.Array,
    B_w_gate: jax.Array,
    B_w_up: jax.Array,
    B_w_down: jax.Array,
):
    del B_x
    B, Sq, D = A_x.shape
    _, H, Sk, Dh = A_k_cache.shape
    F = B_w_gate.shape[1]
    assert (B, Sq, D, H, Sk, Dh, F) == (4, 1, 640, 32, 8192, 192, 1536)
    W = _NS * _RB
    HG = 3 * W // Dh
    dt = A_k_cache.dtype
    f32 = jnp.float32

    kt = jnp.swapaxes(A_k_cache, 2, 3).reshape(B * H * Dh // _RB, _RB, Sk)
    vt = jnp.swapaxes(A_v_cache, 2, 3).reshape(B * H * Dh // _RB, _RB, Sk)

    wq = A_wq.reshape(_WS, D // _WS, H * Dh)
    wo = A_wo.reshape(_WS, H * Dh // _WS, D)
    wd = B_w_down.reshape(_DS, F // _DS, D)

    out = pl.pallas_call(
        functools.partial(_body, B=B, H=H, Dh=Dh, Sk=Sk, D=D, F=F),
        in_specs=[pl.BlockSpec(memory_space=pl.ANY)] * 9,
        out_specs=pl.BlockSpec(memory_space=pltpu.VMEM),
        out_shape=jax.ShapeDtypeStruct((B, D), A_x.dtype),
        scratch_shapes=[
            pltpu.VMEM((2, _NS, _RB, Sk), dt),
            pltpu.VMEM((_WS, D // _WS, H * Dh), dt),
            pltpu.VMEM((_WS, H * Dh // _WS, D), dt),
            pltpu.VMEM((D, F), dt),
            pltpu.VMEM((D, F), dt),
            pltpu.VMEM((_DS, F // _DS, D), dt),
            pltpu.VMEM((B, D), dt),
            pltpu.VMEM((D,), dt),
            pltpu.VMEM((H * Dh // W, 2 * B, W), f32),
            pltpu.VMEM((H * Dh // W, 2 * B, W), f32),
            pltpu.VMEM((HG, W), dt),
            pltpu.VMEM((HG, Sk), f32),
            pltpu.VMEM((HG, Sk), dt),
            pltpu.VMEM((HG, 1), f32),
            pltpu.VMEM((HG, W), f32),
            pltpu.VMEM((2 * B, D), f32),
            pltpu.SemaphoreType.DMA((2,)),
            pltpu.SemaphoreType.DMA((4,)),
            pltpu.SemaphoreType.DMA((2,)),
            pltpu.SemaphoreType.DMA((len(_DP),)),
        ],
        compiler_params=pltpu.CompilerParams(
            vmem_limit_bytes=80 * 1024 * 1024, disable_bounds_checks=True
        ),
    )(A_x.reshape(B, D), kt, vt, wq, wo, B_w_r, B_w_gate, B_w_up, wd)
    return out.reshape(B, Sq, D)
```

```python
import functools

import jax
import jax.numpy as jnp
import jax.experimental.pallas as pl
import jax.experimental.pallas.tpu as pltpu

_EPS = 1e-5
_RB = 64
_NS = 12
_CW = 1024
_MW = 512
_RUNS = (((0, 1), (4, 1), (8, 1)), ((1, 3), (5, 3), (9, 3)))
_STEP = 6
_SKEW = 26
_LAG = 8
_WS = 8
_DP = 256


def _layernorm(x):
    m = jnp.mean(x, axis=-1, keepdims=True)
    d = x - m
    v = jnp.mean(d * d, axis=-1, keepdims=True)
    return d / jnp.sqrt(v + _EPS)


def _dot(a, b):
    return jnp.dot(a, b, preferred_element_type=jnp.float32)


def _dot_nt(a, b):
    return jax.lax.dot_general(
        a, b, (((1,), (1,)), ((), ())), preferred_element_type=jnp.float32
    )


def _wait_all(buf, sem):
    pltpu.make_async_copy(buf, buf, sem).wait()


def _loop(lo, hi, body):
    jax.lax.fori_loop(lo, hi, lambda i, carry: body(i), None)


def _ds(start, size):
    if isinstance(start, int):
        return pl.ds(start, size)
    return pl.ds(pl.multiple_of(start, size), size)


def _start(copies0, copies1):
    for j in range(max(len(copies0), len(copies1))):
        for queue, copies in enumerate((copies0, copies1)):
            if j < len(copies):
                pltpu.make_async_copy(*copies[j]).start(priority=queue)


def _steps(lo, hi, copies, first, second, work):
    whole, rest = divmod(_SKEW, _STEP)

    def step(i):
        _start(copies(i, 0), first(i + whole, 1)[rest:] + second(i + whole + 1, 1)[:rest])
        work(i)

    _loop(lo, hi, step)


def _phase(copies, n, after, work=lambda i: None):
    following = lambda i, queue: after(i - n, queue)
    mid = n - _SKEW // _STEP - 1
    _steps(0, mid, copies, copies, copies, work)
    _steps(mid, mid + 1, copies, copies, following, lambda i: None)
    _steps(mid + 1, n, copies, following, following, lambda i: None)


def _body(
    x_hbm, kt_hbm, vt_hbm, wq_hbm, wo_hbm, wr_hbm, wg_hbm, wu_hbm, wd_hbm,
    out_ref,
    kbuf, vbuf, wqbuf, wobuf, wgbuf, wubuf, wdbuf, xbuf, wrbuf,
    q_scr, o_scr, lhs_scr, s_scr, p_scr, l_scr, acc_scr, h_scr,
    sem, wsem, gsem, dsem,
    *, B, H, Dh, Sk, D, F,
):
    W = _NS * _RB
    NW = H * Dh // W
    NC = Sk // _CW
    NM = Sk // _MW
    visits = _STEP // len(_RUNS[0])
    steps = (_RB // 8) * NC // visits
    scale = Dh ** -0.5

    def cache_copies(src, dst, copy_sem, win, i, queue):
        out = []
        for u in range(visits):
            u = i * visits + u
            rows, cols = _ds((u // NC) * 8, 8), _ds((u % NC) * _CW, _CW)
            for first, n in _RUNS[queue]:
                out.append((
                    src.at[pl.ds(win * _NS + first, n), rows, cols],
                    dst.at[pl.ds(first, n), rows, cols],
                    copy_sem,
                ))
        return out

    def k_copies(win):
        return functools.partial(cache_copies, kt_hbm, kbuf, sem.at[0], win)

    def v_copies(win):
        return functools.partial(cache_copies, vt_hbm, vbuf, sem.at[1], win)

    def wq_copies(i, queue):
        n = H * Dh // _CW
        out = []
        for u in range(_STEP // 2):
            u = i * (_STEP // 2) + u
            for pair in (queue, queue + 2):
                part = (pl.ds(2 * pair, 2), _ds((u // n) * 8, 8), _ds((u % n) * _CW, _CW))
                out.append((wq_hbm.at[part], wqbuf.at[part], wsem.at[2]))
        return out

    def wo_copies(i, queue):
        out = []
        for u in range(_STEP // 2):
            for pair in (queue, queue + 2):
                part = (pl.ds(2 * pair, 2), _ds((i * (_STEP // 2) + u) * 16, 16))
                out.append((wo_hbm.at[part], wobuf.at[part], wsem.at[3]))
        return out

    def gate_up_copies(i, queue):
        src, dst = ((wg_hbm, wgbuf), (wu_hbm, wubuf))[queue]
        out = []
        for u in range(_STEP):
            rows = _ds((u % 2) * (D // 2) + (i * (_STEP // 2) + u // 2) * 8, 8)
            out.append((src.at[rows, :], dst.at[rows, :], gsem.at[queue]))
        return out

    def last_copies(i, queue):
        src, dst = ((wg_hbm, wgbuf), (wu_hbm, wubuf))[queue]
        out = []
        for u in range(i * _STEP, D // 8):
            rows = pl.ds((u % 2) * (D // 2) + u // 2 * 8, 8)
            out.append((src.at[rows, :], dst.at[rows, :], gsem.at[queue]))
        for lo in range(0, F // 2, 32):
            part = (queue, pl.ds(lo, 32))
            out.append((wd_hbm.at[part], wdbuf.at[part], dsem.at[lo // _DP]))
        return out

    def own_head():
        lo = jax.lax.broadcasted_iota(jnp.int32, (2 * B, W), 0) * Dh
        col = jax.lax.broadcasted_iota(jnp.int32, (2 * B, W), 1)
        return (lo <= col) & (col < lo + Dh)

    def consume_k(win, c):
        @pl.when(c == 0)
        def _():
            _wait_all(kbuf, sem.at[0])
            q = q_scr[win % NW, pl.ds(win // NW, 1), :]
            lhs_scr[...] = jnp.where(own_head(), q, 0.0)

        cols = _ds(c * _MW, _MW)
        s_scr[:, cols] = _dot(lhs_scr[...].astype(kbuf.dtype), kbuf[:, :, cols].reshape(W, _MW))

    def softmax():
        s = s_scr[...] * scale
        e = jnp.exp(s - jnp.max(s, axis=-1, keepdims=True))
        l_scr[...] = jnp.sum(e, axis=-1, keepdims=True)
        p_scr[...] = e

    def consume_v(win, c):
        @pl.when(c == 0)
        def _():
            _wait_all(vbuf, sem.at[1])
            acc_scr[...] = jnp.zeros_like(acc_scr)

        cols = _ds(c * _MW, _MW)
        p = p_scr[:, cols].astype(vbuf.dtype)
        acc_scr[...] += _dot_nt(p, vbuf[:, :, cols].reshape(W, _MW))

        @pl.when(c == NM - 1)
        def _():
            o = jnp.where(own_head(), acc_scr[...] / l_scr[...], 0.0)
            o_scr[win % NW, pl.ds(win // NW, 1), :] = jnp.sum(o, axis=0, keepdims=True)

    whole, rest = divmod(_SKEW, _STEP)
    x_cp = pltpu.make_async_copy(x_hbm, xbuf, wsem.at[0])
    wr_cp = pltpu.make_async_copy(wr_hbm, wrbuf, wsem.at[1])
    _loop(0, whole, lambda i: _start([], wq_copies(i, 1)))
    _start([], wq_copies(whole, 1)[:rest])
    x_cp.start()
    wr_cp.start()
    _phase(wq_copies, 2 * (D // _WS // 8) * (H * Dh // _CW) // _STEP, k_copies(0))

    x_cp.wait()
    x4 = xbuf[...].astype(jnp.float32)
    x = jnp.concatenate([x4, x4], axis=0)
    xn = _layernorm(x).astype(jnp.bfloat16)
    h_scr[...] = x
    o_scr[...] = jnp.zeros_like(o_scr)

    def project(w):
        pl.when(w == 0)(lambda: _wait_all(wqbuf, wsem.at[2]))
        q_scr[w] = _dot(xn, wqbuf[:, :, _ds(w * W, W)].reshape(D, W))

    def window(win, after):
        def during_k(i):
            c = i - _LAG
            pl.when((win == 0) & (c >= 0) & (c < NW))(lambda: project(c))
            pl.when((win > 0) & (c >= 0) & (c < NM))(lambda: consume_v(win - 1, c))

        def during_v(i):
            c = i - _LAG
            pl.when((c >= 0) & (c < NM))(lambda: consume_k(win, c))
            pl.when(c == NM)(softmax)

        _phase(k_copies(win), steps, v_copies(win), during_k)
        _phase(v_copies(win), steps, after, during_v)

    last = B * NW - 1
    _loop(0, last, lambda win: window(win, k_copies(win + 1)))
    _loop(last, last + 1, lambda win: window(win, wo_copies))

    def during_wo(i):
        c = 2 * (i - 6)
        pl.when(c >= 0)(lambda: _loop(c, c + 2, lambda c: consume_v(last, c)))

    def during_gate_up(i):
        pl.when(i < 3)(lambda: _loop(10 + 2 * i, 12 + 2 * i, lambda c: consume_v(last, c)))
        pl.when(i == 6)(lambda: _wait_all(wobuf, wsem.at[3]))
        pl.when(i >= 6)(lambda: out_project(i - 6))

    def out_project(j):
        o = jnp.concatenate([o_scr[2 * j], o_scr[2 * j + 1]], axis=1).astype(jnp.bfloat16)
        n = _WS // (NW // 2)
        h_scr[...] += _dot(o, wobuf[pl.ds(j * n, n)].reshape(2 * W, D))

    _phase(wo_copies, 2 * (H * Dh // _WS // 16) // _STEP, gate_up_copies, during_wo)
    _steps(0, 8, gate_up_copies, gate_up_copies, gate_up_copies, during_gate_up)
    end0, end1 = last_copies(8, 0), last_copies(8, 1)[_SKEW:]
    _start(end0[:_STEP], end1[:_STEP])
    _loop(2, NW // 2, out_project)
    _start(end0[_STEP:2 * _STEP], end1[_STEP:2 * _STEP])
    h = h_scr[...]
    hn = _layernorm(h)
    hb = hn.astype(jnp.bfloat16)
    wr_cp.wait()
    r = jnp.sum(hn * wrbuf[...].astype(jnp.float32).reshape(1, D), axis=-1, keepdims=True)
    route = jax.nn.sigmoid(r)
    _start(end0[2 * _STEP:], end1[2 * _STEP:])

    _wait_all(wgbuf, gsem.at[0])
    _wait_all(wubuf, gsem.at[1])
    gate = _dot(hb, wgbuf[...])
    act = (gate * jax.nn.sigmoid(gate) * _dot(hb, wubuf[...])).astype(jnp.bfloat16)
    y = jnp.zeros((2 * B, D), jnp.float32)
    for lo in range(0, F // 2, _DP):
        piece = wdbuf.at[:, pl.ds(lo, _DP), :]
        a = jnp.concatenate([act[:, c + lo:c + lo + _DP] for c in (0, F // 2)], axis=1)
        _wait_all(piece, dsem.at[lo // _DP])
        y = y + _dot(a, piece[...].reshape(2 * _DP, D))
    out = h + (hn + (hn * 0.0 + y * route))
    out_ref[...] = out[:B].astype(out_ref.dtype)


@jax.jit
def pallas_sequential_preLN__mha_block_cached__moe_arch_mod__decode_kernel(
    A_x: jax.Array,
    A_k_cache: jax.Array,
    A_v_cache: jax.Array,
    A_wq: jax.Array,
    A_wo: jax.Array,
    B_x: jax.Array,
    B_w_r: jax.Array,
    B_w_gate: jax.Array,
    B_w_up: jax.Array,
    B_w_down: jax.Array,
):
    del B_x
    B, Sq, D = A_x.shape
    _, H, Sk, Dh = A_k_cache.shape
    F = B_w_gate.shape[1]
    assert (B, Sq, D, H, Sk, Dh, F) == (4, 1, 640, 32, 8192, 192, 1536)
    W = _NS * _RB
    dt = A_k_cache.dtype
    f32 = jnp.float32

    kt = jnp.swapaxes(A_k_cache, 2, 3).reshape(B * H * Dh // _RB, _RB, Sk)
    vt = jnp.swapaxes(A_v_cache, 2, 3).reshape(B * H * Dh // _RB, _RB, Sk)
    wq = A_wq.reshape(_WS, D // _WS, H * Dh)
    wo = A_wo.reshape(_WS, H * Dh // _WS, D)
    wd = B_w_down.reshape(2, F // 2, D)

    out = pl.pallas_call(
        functools.partial(_body, B=B, H=H, Dh=Dh, Sk=Sk, D=D, F=F),
        in_specs=[pl.BlockSpec(memory_space=pl.ANY)] * 9,
        out_specs=pl.BlockSpec(memory_space=pltpu.VMEM),
        out_shape=jax.ShapeDtypeStruct((B, D), A_x.dtype),
        scratch_shapes=[
            pltpu.VMEM((_NS, _RB, Sk), dt),
            pltpu.VMEM((_NS, _RB, Sk), dt),
            pltpu.VMEM(wq.shape, dt),
            pltpu.VMEM(wo.shape, dt),
            pltpu.VMEM((D, F), dt),
            pltpu.VMEM((D, F), dt),
            pltpu.VMEM(wd.shape, dt),
            pltpu.VMEM((B, D), dt),
            pltpu.VMEM((D,), dt),
            pltpu.VMEM((H * Dh // W, 2 * B, W), f32),
            pltpu.VMEM((H * Dh // W, 2 * B, W), f32),
            pltpu.VMEM((2 * B, W), f32),
            pltpu.VMEM((2 * B, Sk), f32),
            pltpu.VMEM((2 * B, Sk), f32),
            pltpu.VMEM((2 * B, 1), f32),
            pltpu.VMEM((2 * B, W), f32),
            pltpu.VMEM((2 * B, D), f32),
            pltpu.SemaphoreType.DMA((2,)),
            pltpu.SemaphoreType.DMA((4,)),
            pltpu.SemaphoreType.DMA((2,)),
            pltpu.SemaphoreType.DMA((F // 2 // _DP,)),
        ],
        compiler_params=pltpu.CompilerParams(
            vmem_limit_bytes=64 * 1024 * 1024, disable_bounds_checks=True
        ),
    )(A_x.reshape(B, D), kt, vt, wq, wo, B_w_r, B_w_gate, B_w_up, wd)
    return out.reshape(B, Sq, D)
```

```python
import functools

import jax
import jax.numpy as jnp
import jax.experimental.pallas as pl
import jax.experimental.pallas.tpu as pltpu

_EPS = 1e-5
_RB = 64
_NS = 12
_CW = 1024
_MW = 512
_RUNS = (((0, 1), (4, 1), (8, 1)), ((1, 3), (5, 3), (9, 3)))
_STEP = 6
_SKEW = 26
_LAG = 8
_WS = 8
_DS = 4
_DP = (96, 192, 320, 384)


def _layernorm(x):
    m = jnp.mean(x, axis=-1, keepdims=True)
    d = x - m
    v = jnp.mean(d * d, axis=-1, keepdims=True)
    return d / jnp.sqrt(v + _EPS)


def _dot(a, b):
    return jnp.dot(a, b, preferred_element_type=jnp.float32)


def _dot_nt(a, b):
    return jax.lax.dot_general(
        a, b, (((1,), (1,)), ((), ())), preferred_element_type=jnp.float32
    )


def _wait_all(buf, sem):
    pltpu.make_async_copy(buf, buf, sem).wait()


def _loop(lo, hi, body):
    jax.lax.fori_loop(lo, hi, lambda i, carry: body(i), None)


def _ds(start, size):
    if isinstance(start, int):
        return pl.ds(start, size)
    return pl.ds(pl.multiple_of(start, size), size)


def _start(copies0, copies1):
    for j in range(max(len(copies0), len(copies1))):
        for queue, copies in enumerate((copies0, copies1)):
            if j < len(copies):
                pltpu.make_async_copy(*copies[j]).start(priority=queue)


def _steps(lo, hi, copies, first, second, work):
    whole, rest = divmod(_SKEW, _STEP)

    def step(i):
        _start(copies(i, 0), first(i + whole, 1)[rest:] + second(i + whole + 1, 1)[:rest])
        work(i)

    _loop(lo, hi, step)


def _phase(copies, n, after, work=lambda i: None):
    following = lambda i, queue: after(i - n, queue)
    mid = n - _SKEW // _STEP - 1
    _steps(0, mid, copies, copies, copies, work)
    _steps(mid, mid + 1, copies, copies, following, lambda i: None)
    _steps(mid + 1, n, copies, following, following, lambda i: None)


def _body(
    x_hbm, kt_hbm, vt_hbm, wq_hbm, wo_hbm, wr_hbm, wg_hbm, wu_hbm, wd_hbm,
    out_ref,
    kbuf, vbuf, wqbuf, wobuf, wgbuf, wubuf, wdbuf, xbuf, wrbuf,
    q_scr, o_scr, lhs_scr, s_scr, p_scr, l_scr, acc_scr, h_scr,
    sem, wsem, gsem, dsem,
    *, B, H, Dh, Sk, D, F,
):
    W = _NS * _RB
    NW = H * Dh // W
    NC = Sk // _CW
    NM = Sk // _MW
    visits = _STEP // len(_RUNS[0])
    steps = (_RB // 8) * NC // visits
    scale = Dh ** -0.5

    def cache_copies(src, dst, copy_sem, win, i, queue):
        out = []
        for u in range(visits):
            u = i * visits + u
            rows, cols = _ds((u // NC) * 8, 8), _ds((u % NC) * _CW, _CW)
            for first, n in _RUNS[queue]:
                out.append((
                    src.at[pl.ds(win * _NS + first, n), rows, cols],
                    dst.at[pl.ds(first, n), rows, cols],
                    copy_sem,
                ))
        return out

    def k_copies(win):
        return functools.partial(cache_copies, kt_hbm, kbuf, sem.at[0], win)

    def v_copies(win):
        return functools.partial(cache_copies, vt_hbm, vbuf, sem.at[1], win)

    def wq_copies(i, queue):
        n = H * Dh // _CW
        out = []
        for u in range(_STEP // 2):
            u = i * (_STEP // 2) + u
            for pair in (2 * queue, 2 * queue + 1):
                part = (pl.ds(2 * pair, 2), _ds((u // n) * 8, 8), _ds((u % n) * _CW, _CW))
                out.append((wq_hbm.at[part], wqbuf.at[part], wsem.at[2]))
        return out

    def wo_copies(i, queue):
        out = []
        for u in range(_STEP // 2):
            for pair in (queue, queue + 2):
                part = (pl.ds(2 * pair, 2), _ds((i * (_STEP // 2) + u) * 16, 16))
                out.append((wo_hbm.at[part], wobuf.at[part], wsem.at[3]))
        return out

    def gate_up_copies(i, queue):
        src, dst = ((wg_hbm, wgbuf), (wu_hbm, wubuf))[queue]
        out = []
        for u in range(_STEP):
            u = i * _STEP + u
            rows = _ds((u % 4) * (D // 4) + u // 4 * 8, 8)
            out.append((src.at[rows, :], dst.at[rows, :], gsem.at[queue]))
        return out

    def last_copies(i, queue):
        src, dst = ((wg_hbm, wgbuf), (wu_hbm, wubuf))[queue]
        out = []
        for u in range(i * _STEP, D // 8):
            rows = pl.ds((u % 4) * (D // 4) + u // 4 * 8, 8)
            out.append((src.at[rows, :], dst.at[rows, :], gsem.at[queue]))
        streams = pl.ds(queue * _DS // 4, (1 + 2 * queue) * _DS // 4)
        for lo in range(0, F // _DS, 64 // _DS):
            part = (streams, pl.ds(lo, 64 // _DS))
            piece = sum(lo >= end for end in _DP)
            out.append((wd_hbm.at[part], wdbuf.at[part], dsem.at[piece]))
        return out

    def own_head():
        lo = jax.lax.broadcasted_iota(jnp.int32, (2 * B, W), 0) * Dh
        col = jax.lax.broadcasted_iota(jnp.int32, (2 * B, W), 1)
        return (lo <= col) & (col < lo + Dh)

    def consume_k(win, c):
        @pl.when(c == 0)
        def _():
            _wait_all(kbuf, sem.at[0])
            q = q_scr[win % NW, pl.ds(win // NW, 1), :]
            lhs_scr[...] = jnp.where(own_head(), q, 0.0)

        cols = _ds(c * _MW, _MW)
        s_scr[:, cols] = _dot(lhs_scr[...].astype(kbuf.dtype), kbuf[:, :, cols].reshape(W, _MW))

    def softmax():
        s = s_scr[...] * scale
        e = jnp.exp(s - jnp.max(s, axis=-1, keepdims=True))
        l_scr[...] = jnp.sum(e, axis=-1, keepdims=True)
        p_scr[...] = e

    def consume_v(win, c):
        @pl.when(c == 0)
        def _():
            _wait_all(vbuf, sem.at[1])
            acc_scr[...] = jnp.zeros_like(acc_scr)

        cols = _ds(c * _MW, _MW)
        p = p_scr[:, cols].astype(vbuf.dtype)
        acc_scr[...] += _dot_nt(p, vbuf[:, :, cols].reshape(W, _MW))

        @pl.when(c == NM - 1)
        def _():
            o = jnp.where(own_head(), acc_scr[...] / l_scr[...], 0.0)
            o_scr[win % NW, pl.ds(win // NW, 1), :] = jnp.sum(o, axis=0, keepdims=True)

    whole, rest = divmod(_SKEW, _STEP)
    x_cp = pltpu.make_async_copy(x_hbm, xbuf, wsem.at[0])
    wr_cp = pltpu.make_async_copy(wr_hbm, wrbuf, wsem.at[1])
    _loop(0, whole, lambda i: _start([], wq_copies(i, 1)))
    _start([], wq_copies(whole, 1)[:rest])
    x_cp.start()
    wr_cp.start()
    _phase(wq_copies, 2 * (D // _WS // 8) * (H * Dh // _CW) // _STEP, k_copies(0))

    x_cp.wait()
    x4 = xbuf[...].astype(jnp.float32)
    x = jnp.concatenate([x4, x4], axis=0)
    xn = _layernorm(x).astype(jnp.bfloat16)
    h_scr[...] = x
    o_scr[...] = jnp.zeros_like(o_scr)

    def project(w):
        pl.when(w == 0)(lambda: _wait_all(wqbuf, wsem.at[2]))
        q_scr[w] = _dot(xn, wqbuf[:, :, _ds(w * W, W)].reshape(D, W))

    def window(win, after):
        def during_k(i):
            c = i - _LAG
            pl.when((win == 0) & (c >= 0) & (c < NW))(lambda: project(c))
            pl.when((win > 0) & (c >= 0) & (c < NM))(lambda: consume_v(win - 1, c))

        def during_v(i):
            c = i - _LAG
            pl.when((c >= 0) & (c < NM))(lambda: consume_k(win, c))
            pl.when(c == NM)(softmax)

        _phase(k_copies(win), steps, v_copies(win), during_k)
        _phase(v_copies(win), steps, after, during_v)

    last = B * NW - 1
    _loop(0, last, lambda win: window(win, k_copies(win + 1)))
    _loop(last, last + 1, lambda win: window(win, wo_copies))

    def during_wo(i):
        c = 2 * (i - 6)
        pl.when(c >= 0)(lambda: _loop(c, c + 2, lambda c: consume_v(last, c)))

    def during_gate_up(i):
        pl.when(i < 3)(lambda: _loop(10 + 2 * i, 12 + 2 * i, lambda c: consume_v(last, c)))
        pl.when(i == 6)(lambda: _wait_all(wobuf, wsem.at[3]))
        pl.when(i >= 6)(lambda: out_project(i - 6))

    def out_project(j):
        o = jnp.concatenate([o_scr[2 * j], o_scr[2 * j + 1]], axis=1).astype(jnp.bfloat16)
        n = _WS // (NW // 2)
        h_scr[...] += _dot(o, wobuf[pl.ds(j * n, n)].reshape(2 * W, D))

    _phase(wo_copies, 2 * (H * Dh // _WS // 16) // _STEP, gate_up_copies, during_wo)
    _steps(0, 8, gate_up_copies, gate_up_copies, gate_up_copies, during_gate_up)
    end0, end1 = last_copies(8, 0), last_copies(8, 1)[_SKEW:]
    _start(end0[:_STEP], end1[:_STEP])
    _loop(2, NW // 2, out_project)
    _start(end0[_STEP:2 * _STEP], end1[_STEP:2 * _STEP])
    h = h_scr[...]
    hn = _layernorm(h)
    hb = hn.astype(jnp.bfloat16)
    wr_cp.wait()
    r = jnp.sum(hn * wrbuf[...].astype(jnp.float32).reshape(1, D), axis=-1, keepdims=True)
    route = jax.nn.sigmoid(r)
    _start(end0[2 * _STEP:], end1[2 * _STEP:])

    _wait_all(wgbuf, gsem.at[0])
    _wait_all(wubuf, gsem.at[1])
    gate = _dot(hb, wgbuf[...])
    act = gate * jax.nn.sigmoid(gate) * _dot(hb, wubuf[...])
    pieces = [
        (lo, hi, jnp.concatenate([act[:, c + lo:c + hi] for c in range(0, F, F // _DS)], axis=1))
        for lo, hi in zip((0,) + _DP, _DP)
    ]
    y = jnp.zeros((2 * B, D), jnp.float32)
    for i, (lo, hi, a) in enumerate(pieces):
        piece = wdbuf.at[:, pl.ds(lo, hi - lo), :]
        a = a.astype(jnp.bfloat16)
        _wait_all(piece, dsem.at[i])
        y = y + _dot(a, piece[...].reshape(_DS * (hi - lo), D))
    out = h + (hn + (hn * 0.0 + y * route))
    out_ref[...] = out[:B].astype(out_ref.dtype)


@jax.jit
def pallas_sequential_preLN__mha_block_cached__moe_arch_mod__decode_kernel(
    A_x: jax.Array,
    A_k_cache: jax.Array,
    A_v_cache: jax.Array,
    A_wq: jax.Array,
    A_wo: jax.Array,
    B_x: jax.Array,
    B_w_r: jax.Array,
    B_w_gate: jax.Array,
    B_w_up: jax.Array,
    B_w_down: jax.Array,
):
    del B_x
    B, Sq, D = A_x.shape
    _, H, Sk, Dh = A_k_cache.shape
    F = B_w_gate.shape[1]
    assert (B, Sq, D, H, Sk, Dh, F) == (4, 1, 640, 32, 8192, 192, 1536)
    W = _NS * _RB
    dt = A_k_cache.dtype
    f32 = jnp.float32

    kt = jnp.swapaxes(A_k_cache, 2, 3).reshape(B * H * Dh // _RB, _RB, Sk)
    vt = jnp.swapaxes(A_v_cache, 2, 3).reshape(B * H * Dh // _RB, _RB, Sk)
    wq = A_wq.reshape(_WS, D // _WS, H * Dh)
    wo = A_wo.reshape(_WS, H * Dh // _WS, D)
    wd = B_w_down.reshape(_DS, F // _DS, D)

    out = pl.pallas_call(
        functools.partial(_body, B=B, H=H, Dh=Dh, Sk=Sk, D=D, F=F),
        in_specs=[pl.BlockSpec(memory_space=pl.ANY)] * 9,
        out_specs=pl.BlockSpec(memory_space=pltpu.VMEM),
        out_shape=jax.ShapeDtypeStruct((B, D), A_x.dtype),
        scratch_shapes=[
            pltpu.VMEM((_NS, _RB, Sk), dt),
            pltpu.VMEM((_NS, _RB, Sk), dt),
            pltpu.VMEM(wq.shape, dt),
            pltpu.VMEM(wo.shape, dt),
            pltpu.VMEM((D, F), dt),
            pltpu.VMEM((D, F), dt),
            pltpu.VMEM(wd.shape, dt),
            pltpu.VMEM((B, D), dt),
            pltpu.VMEM((D,), dt),
            pltpu.VMEM((H * Dh // W, 2 * B, W), f32),
            pltpu.VMEM((H * Dh // W, 2 * B, W), f32),
            pltpu.VMEM((2 * B, W), f32),
            pltpu.VMEM((2 * B, Sk), f32),
            pltpu.VMEM((2 * B, Sk), f32),
            pltpu.VMEM((2 * B, 1), f32),
            pltpu.VMEM((2 * B, W), f32),
            pltpu.VMEM((2 * B, D), f32),
            pltpu.SemaphoreType.DMA((2,)),
            pltpu.SemaphoreType.DMA((4,)),
            pltpu.SemaphoreType.DMA((2,)),
            pltpu.SemaphoreType.DMA((len(_DP),)),
        ],
        compiler_params=pltpu.CompilerParams(vmem_limit_bytes=64 * 1024 * 1024),
    )(A_x.reshape(B, D), kt, vt, wq, wo, B_w_r, B_w_gate, B_w_up, wd)
    return out.reshape(B, Sq, D)
```

```python
import functools

import jax
import jax.numpy as jnp
import jax.experimental.pallas as pl
import jax.experimental.pallas.tpu as pltpu

_EPS = 1e-5
_RB = 64
_NS = 12
_CW = 1024
_MW = 512
_RUNS = (((0, 1), (4, 1), (8, 1)), ((1, 3), (5, 3), (9, 3)))
_STEP = 6
_SKEW = 26
_LAG = 8
_QB = 128
_WS = 8
_DS = 4
_DP = (96, 192, 320, 384)


def _layernorm(x):
    m = jnp.mean(x, axis=-1, keepdims=True)
    d = x - m
    v = jnp.mean(d * d, axis=-1, keepdims=True)
    return d / jnp.sqrt(v + _EPS)


def _dot(a, b):
    return jnp.dot(a, b, preferred_element_type=jnp.float32)


def _dot_nt(a, b):
    return jax.lax.dot_general(
        a, b, (((1,), (1,)), ((), ())), preferred_element_type=jnp.float32
    )


def _wait_all(buf, sem):
    pltpu.make_async_copy(buf, buf, sem).wait()


def _loop(lo, hi, body):
    jax.lax.fori_loop(lo, hi, lambda i, carry: body(i), None)


def _ds(start, size):
    if isinstance(start, int):
        return pl.ds(start, size)
    return pl.ds(pl.multiple_of(start, size), size)


def _start(copies0, copies1):
    for j in range(max(len(copies0), len(copies1))):
        for queue, copies in enumerate((copies0, copies1)):
            if j < len(copies):
                pltpu.make_async_copy(*copies[j]).start(priority=queue)


def _steps(lo, hi, copies, first, second, work):
    whole, rest = divmod(_SKEW, _STEP)

    def step(i):
        _start(copies(i, 0), first(i + whole, 1)[rest:] + second(i + whole + 1, 1)[:rest])
        work(i)

    _loop(lo, hi, step)


def _phase(copies, n, after, work=lambda i: None):
    following = lambda i, queue: after(i - n, queue)
    mid = n - _SKEW // _STEP - 1
    _steps(0, mid, copies, copies, copies, work)
    _steps(mid, mid + 1, copies, copies, following, lambda i: None)
    _steps(mid + 1, n, copies, following, following, lambda i: None)


def _body(
    x_hbm, kt_hbm, vt_hbm, wq_hbm, wo_hbm, wr_hbm, wg_hbm, wu_hbm, wd_hbm,
    out_ref,
    kbuf, vbuf, wqbuf, wobuf, wgbuf, wubuf, wdbuf, xbuf, wrbuf,
    q_scr, o_scr, lhs_scr, s_scr, p_scr, l_scr, acc_scr, h_scr,
    sem, wsem, gsem, dsem,
    *, B, H, Dh, Sk, D, F,
):
    W = _NS * _RB
    NW = H * Dh // W
    NC = Sk // _CW
    NM = Sk // _MW
    visits = _STEP // len(_RUNS[0])
    steps = (_RB // 8) * NC // visits
    wq_visits = (_QB // 8) * (H * Dh // _CW) // 3
    scale = Dh ** -0.5

    def cache_copies(src, dst, copy_sem, win, i, queue):
        out = []
        for u in range(visits):
            u = i * visits + u
            rows, cols = _ds((u // NC) * 8, 8), _ds((u % NC) * _CW, _CW)
            for first, n in _RUNS[queue]:
                out.append((
                    src.at[pl.ds(win * _NS + first, n), rows, cols],
                    dst.at[pl.ds(first, n), rows, cols],
                    copy_sem,
                ))
        return out

    def k_copies(win):
        return functools.partial(cache_copies, kt_hbm, kbuf, sem.at[0], win)

    def v_copies(win):
        return functools.partial(cache_copies, vt_hbm, vbuf, sem.at[1], win)

    def wq_copies(i, queue):
        n = H * Dh // _CW
        blocks = (pl.ds(0, 1), pl.ds(1, D // _QB - 1))[queue]
        out = []
        for u in range(_STEP // 3):
            for j in range(3):
                p = i * (_STEP // 3) + u + j * wq_visits
                part = (blocks, _ds((p // n) * 8, 8), _ds((p % n) * _CW, _CW))
                out.append((wq_hbm.at[part], wqbuf.at[part], wsem.at[2]))
        return out

    def wo_copies(i, queue):
        out = []
        for u in range(_STEP // 2):
            for pair in (queue, queue + 2):
                part = (pl.ds(2 * pair, 2), _ds((i * (_STEP // 2) + u) * 16, 16))
                out.append((wo_hbm.at[part], wobuf.at[part], wsem.at[3]))
        return out

    def gate_up_copies(i, queue):
        src, dst = ((wg_hbm, wgbuf), (wu_hbm, wubuf))[queue]
        out = []
        for u in range(_STEP):
            u = i * _STEP + u
            rows = _ds((u % 4) * (D // 4) + u // 4 * 8, 8)
            out.append((src.at[rows, :], dst.at[rows, :], gsem.at[queue]))
        return out

    def last_copies(i, queue):
        src, dst = ((wg_hbm, wgbuf), (wu_hbm, wubuf))[queue]
        out = []
        for u in range(i * _STEP, D // 8):
            rows = pl.ds((u % 4) * (D // 4) + u // 4 * 8, 8)
            out.append((src.at[rows, :], dst.at[rows, :], gsem.at[queue]))
        streams = pl.ds(queue * _DS // 4, (1 + 2 * queue) * _DS // 4)
        for lo in range(0, F // _DS, 64 // _DS):
            part = (streams, pl.ds(lo, 64 // _DS))
            piece = sum(lo >= end for end in _DP)
            out.append((wd_hbm.at[part], wdbuf.at[part], dsem.at[piece]))
        return out

    def own_head():
        lo = jax.lax.broadcasted_iota(jnp.int32, (2 * B, W), 0) * Dh
        col = jax.lax.broadcasted_iota(jnp.int32, (2 * B, W), 1)
        return (lo <= col) & (col < lo + Dh)

    def consume_k(win, c):
        @pl.when(c == 0)
        def _():
            _wait_all(kbuf, sem.at[0])
            q = q_scr[win % NW, pl.ds(win // NW, 1), :]
            lhs_scr[...] = jnp.where(own_head(), q, 0.0)

        cols = _ds(c * _MW, _MW)
        s_scr[:, cols] = _dot(lhs_scr[...].astype(kbuf.dtype), kbuf[:, :, cols].reshape(W, _MW))

    def softmax():
        s = s_scr[...] * scale
        e = jnp.exp(s - jnp.max(s, axis=-1, keepdims=True))
        l_scr[...] = jnp.sum(e, axis=-1, keepdims=True)
        p_scr[...] = e

    def consume_v(win, c):
        @pl.when(c == 0)
        def _():
            _wait_all(vbuf, sem.at[1])
            acc_scr[...] = jnp.zeros_like(acc_scr)

        cols = _ds(c * _MW, _MW)
        p = p_scr[:, cols].astype(vbuf.dtype)
        acc_scr[...] += _dot_nt(p, vbuf[:, :, cols].reshape(W, _MW))

        @pl.when(c == NM - 1)
        def _():
            o = jnp.where(own_head(), acc_scr[...] / l_scr[...], 0.0)
            o_scr[win % NW, pl.ds(win // NW, 1), :] = jnp.sum(o, axis=0, keepdims=True)

    whole, rest = divmod(_SKEW, _STEP)
    x_cp = pltpu.make_async_copy(x_hbm, xbuf, wsem.at[0])
    wr_cp = pltpu.make_async_copy(wr_hbm, wrbuf, wsem.at[1])
    x_cp.start()
    wr_cp.start()
    _loop(0, whole, lambda i: _start([], wq_copies(i, 1)))
    _start([], wq_copies(whole, 1)[:rest])
    _phase(wq_copies, 3 * wq_visits // _STEP, k_copies(0))

    x_cp.wait()
    x4 = xbuf[...].astype(jnp.float32)
    x = jnp.concatenate([x4, x4], axis=0)
    xn = _layernorm(x).astype(jnp.bfloat16)
    h_scr[...] = x
    o_scr[...] = jnp.zeros_like(o_scr)

    def project(w):
        pl.when(w == 0)(lambda: _wait_all(wqbuf, wsem.at[2]))
        q_scr[w] = _dot(xn, wqbuf[:, :, _ds(w * W, W)].reshape(D, W))

    def window(win, after):
        def during_k(i):
            c = i - _LAG
            pl.when((win == 0) & (c >= 0) & (c < NW))(lambda: project(c))
            pl.when((win > 0) & (c >= 0) & (c < NM))(lambda: consume_v(win - 1, c))

        def during_v(i):
            c = i - _LAG
            pl.when((c >= 0) & (c < NM))(lambda: consume_k(win, c))
            pl.when(c == NM)(softmax)

        _phase(k_copies(win), steps, v_copies(win), during_k)
        _phase(v_copies(win), steps, after, during_v)

    last = B * NW - 1
    _loop(0, last, lambda win: window(win, k_copies(win + 1)))
    _loop(last, last + 1, lambda win: window(win, wo_copies))

    def during_wo(i):
        c = 2 * (i - 6)
        pl.when(c >= 0)(lambda: _loop(c, c + 2, lambda c: consume_v(last, c)))

    def during_gate_up(i):
        pl.when(i < 3)(lambda: _loop(10 + 2 * i, 12 + 2 * i, lambda c: consume_v(last, c)))
        pl.when(i == 6)(lambda: _wait_all(wobuf, wsem.at[3]))
        pl.when(i >= 6)(lambda: out_project(i - 6))

    def out_project(j):
        o = jnp.concatenate([o_scr[2 * j], o_scr[2 * j + 1]], axis=1).astype(jnp.bfloat16)
        n = _WS // (NW // 2)
        h_scr[...] += _dot(o, wobuf[pl.ds(j * n, n)].reshape(2 * W, D))

    _phase(wo_copies, 2 * (H * Dh // _WS // 16) // _STEP, gate_up_copies, during_wo)
    _steps(0, 8, gate_up_copies, gate_up_copies, gate_up_copies, during_gate_up)
    end0, end1 = last_copies(8, 0), last_copies(8, 1)[_SKEW:]
    _start(end0[:_STEP], end1[:_STEP])
    _loop(2, NW // 2, out_project)
    _start(end0[_STEP:2 * _STEP], end1[_STEP:2 * _STEP])
    h = h_scr[...]
    hn = _layernorm(h)
    hb = hn.astype(jnp.bfloat16)
    wr_cp.wait()
    r = jnp.sum(hn * wrbuf[...].astype(jnp.float32).reshape(1, D), axis=-1, keepdims=True)
    route = jax.nn.sigmoid(r)
    _start(end0[2 * _STEP:], end1[2 * _STEP:])

    _wait_all(wgbuf, gsem.at[0])
    _wait_all(wubuf, gsem.at[1])
    gate = _dot(hb, wgbuf[...])
    act = gate * jax.nn.sigmoid(gate) * _dot(hb, wubuf[...])
    pieces = [
        (lo, hi, jnp.concatenate([act[:, c + lo:c + hi] for c in range(0, F, F // _DS)], axis=1))
        for lo, hi in zip((0,) + _DP, _DP)
    ]
    y = jnp.zeros((2 * B, D), jnp.float32)
    for i, (lo, hi, a) in enumerate(pieces):
        piece = wdbuf.at[:, pl.ds(lo, hi - lo), :]
        a = a.astype(jnp.bfloat16)
        _wait_all(piece, dsem.at[i])
        y = y + _dot(a, piece[...].reshape(_DS * (hi - lo), D))
    out = h + (hn + (hn * 0.0 + y * route))
    out_ref[...] = out[:B].astype(out_ref.dtype)


@jax.jit
def pallas_sequential_preLN__mha_block_cached__moe_arch_mod__decode_kernel(
    A_x: jax.Array,
    A_k_cache: jax.Array,
    A_v_cache: jax.Array,
    A_wq: jax.Array,
    A_wo: jax.Array,
    B_x: jax.Array,
    B_w_r: jax.Array,
    B_w_gate: jax.Array,
    B_w_up: jax.Array,
    B_w_down: jax.Array,
):
    del B_x
    B, Sq, D = A_x.shape
    _, H, Sk, Dh = A_k_cache.shape
    F = B_w_gate.shape[1]
    assert (B, Sq, D, H, Sk, Dh, F) == (4, 1, 640, 32, 8192, 192, 1536)
    W = _NS * _RB
    dt = A_k_cache.dtype
    f32 = jnp.float32

    kt = jnp.swapaxes(A_k_cache, 2, 3).reshape(B * H * Dh // _RB, _RB, Sk)
    vt = jnp.swapaxes(A_v_cache, 2, 3).reshape(B * H * Dh // _RB, _RB, Sk)
    wq = A_wq.reshape(D // _QB, _QB, H * Dh)
    wo = A_wo.reshape(_WS, H * Dh // _WS, D)
    wd = B_w_down.reshape(_DS, F // _DS, D)

    out = pl.pallas_call(
        functools.partial(_body, B=B, H=H, Dh=Dh, Sk=Sk, D=D, F=F),
        in_specs=[pl.BlockSpec(memory_space=pl.ANY)] * 9,
        out_specs=pl.BlockSpec(memory_space=pltpu.VMEM),
        out_shape=jax.ShapeDtypeStruct((B, D), A_x.dtype),
        scratch_shapes=[
            pltpu.VMEM((_NS, _RB, Sk), dt),
            pltpu.VMEM((_NS, _RB, Sk), dt),
            pltpu.VMEM(wq.shape, dt),
            pltpu.VMEM(wo.shape, dt),
            pltpu.VMEM((D, F), dt),
            pltpu.VMEM((D, F), dt),
            pltpu.VMEM(wd.shape, dt),
            pltpu.VMEM((B, D), dt),
            pltpu.VMEM((D,), dt),
            pltpu.VMEM((H * Dh // W, 2 * B, W), f32),
            pltpu.VMEM((H * Dh // W, 2 * B, W), f32),
            pltpu.VMEM((2 * B, W), f32),
            pltpu.VMEM((2 * B, Sk), f32),
            pltpu.VMEM((2 * B, Sk), f32),
            pltpu.VMEM((2 * B, 1), f32),
            pltpu.VMEM((2 * B, W), f32),
            pltpu.VMEM((2 * B, D), f32),
            pltpu.SemaphoreType.DMA((2,)),
            pltpu.SemaphoreType.DMA((4,)),
            pltpu.SemaphoreType.DMA((2,)),
            pltpu.SemaphoreType.DMA((len(_DP),)),
        ],
        compiler_params=pltpu.CompilerParams(vmem_limit_bytes=64 * 1024 * 1024),
    )(A_x.reshape(B, D), kt, vt, wq, wo, B_w_r, B_w_gate, B_w_up, wd)
    return out.reshape(B, Sq, D)
```
